```python
import jax
import jax.numpy as jnp

def _softmax(x, axis=-1):
    return jax.nn.softmax(x, axis=axis)
def _gelu(x):
    return jax.nn.gelu(x, approximate=True)
def _silu(x):
    return jax.nn.silu(x)
def _sigmoid(x):
    return jax.nn.sigmoid(x)
def _layernorm(x, axis=-1, eps=1e-5):
    m = jnp.mean(x, axis=axis, keepdims=True)
    v = jnp.var(x, axis=axis, keepdims=True)
    return (x - m) / jnp.sqrt(v + eps)
def _scatter_add(tgt, idx, src, axis=0):
    return tgt.at[idx].add(src)
def _segment_sum(src, seg, n):
    return jax.ops.segment_sum(src, seg, n)
class _Rng:
    def __init__(self, key):
        self._k = key
    def _next(self):
        self._k, sub = jax.random.split(self._k)
        return sub
    def normal(self, shape):
        return jax.random.normal(self._next(), shape, dtype=jnp.bfloat16)
    def randint(self, lo, hi, shape):
        return jax.random.randint(self._next(), shape, lo, hi, dtype=jnp.int32)
    def uniform(self, shape, lo=0.0, hi=1.0):
        return jax.random.uniform(self._next(), shape, jnp.bfloat16, lo, hi)
    def permutation(self, n):
        return jax.random.permutation(self._next(), n)


kernel_name = 'concat_heads__linear_attn_block__ssm_conv_h3__prompt'

def setup_inputs():
    _rng = _Rng(jax.random.key(int.from_bytes(__import__("os").urandom(4), "little")))
    _w = (lambda a: (lambda t: t.astype(jnp.bfloat16) if jnp.issubdtype(t.dtype, jnp.floating) else t)(jnp.asarray(a)))
    def _A_setup():
        B, S, D = 1, 2048, 1024
        return {
            "x": _w((lambda *s: _rng.normal(s) * 0.05)(B, S, D)),
            "wqkv": _w((lambda *s: _rng.normal(s) * 0.05)(D, 3 * D)),
            "wo": _w((lambda *s: _rng.normal(s) * 0.05)(D, D)),
        }
    _A_in = _A_setup()

    def _B_setup():
        B, S, D = 1, 2048, 1024
        ks = 4
        return {
            "q": _w((lambda *s: _rng.normal(s) * 0.05)(B, S, D)),
            "k": _w((lambda *s: _rng.normal(s) * 0.05)(B, S, D)),
            "v": _w((lambda *s: _rng.normal(s) * 0.05)(B, S, D)),
            "shift_k": _w((lambda *s: _rng.normal(s) * 0.05)(D, ks) * 0.5),
            "ssm_k": _w((lambda *s: _rng.normal(s) * 0.05)(D, S) * (1.0 / S ** 0.5)),
            "ssm_D": _w((lambda *s: _rng.normal(s) * 0.05)(D)),
        }
    _B_in = _B_setup()

    return {
        "A_x": _A_in["x"],
        "A_wqkv": _A_in["wqkv"],
        "A_wo": _A_in["wo"],
        "B_q": _B_in["q"],
        "B_k": _B_in["k"],
        "B_v": _B_in["v"],
        "B_shift_k": _B_in["shift_k"],
        "B_ssm_k": _B_in["ssm_k"],
        "B_ssm_D": _B_in["ssm_D"],
    }

def reference(A_x, A_wqkv, A_wo, B_q, B_k, B_v, B_shift_k, B_ssm_k, B_ssm_D):
    def _A_ref(x, wqkv, wo):
        B, S, D = x.shape
        H = 32; Dh = D // H
        qkv = (lambda x, *d: x.transpose(*d))((x @ wqkv).reshape(B, S, 3, H, Dh), 2, 0, 3, 1, 4)
        q, k, v = qkv[0], qkv[1], qkv[2]
        phi = lambda t: jnp.where(t > 0, t + 1, jnp.exp(t)) + 1e-6
        pq, pk = phi(q), phi(k)
        kv = jnp.einsum("bhsd,bhse->bhde", pk, v)
        z = jnp.einsum("bhsd->bhd", pk)
        num = jnp.einsum("bhqd,bhde->bhqe", pq, kv)
        den = jnp.einsum("bhqd,bhd->bhq", pq, z)[..., None] + 1e-6
        o = num / den
        return (lambda x, *d: x.transpose(*d))(o, 0, 2, 1, 3).reshape(B, S, D) @ wo

    def _B_ref(q, k, v, shift_k, ssm_k, ssm_D):
        B, S, D = q.shape
        ks = shift_k.shape[-1]
        k_pad = jnp.pad(k, ((0, 0), (ks - 1, 0), (0, 0)))
        k_shift = jnp.zeros_like(k)
        for t in range(ks):
            k_shift = k_shift + k_pad[:, t:t + S, :] * shift_k[:, ks - 1 - t][None, None, :]
        kv = k_shift * v
        L = 2 * S
        kv_pad = jnp.pad(kv, ((0, 0), (0, S), (0, 0)))
        kf_pad = jnp.pad(ssm_k, ((0, 0), (0, S)))
        kv_f = (lambda x, axes=(-2,-1): jnp.fft.rfft2(x.astype(jnp.float32), axes=axes))(kv_pad[:, None, :, :], axes=(1, 2))
        kf_f = (lambda x, axes=(-2,-1): jnp.fft.rfft2(x.astype(jnp.float32), axes=axes))(kf_pad[:, None, :], axes=(1, 2))
        kf_f = (lambda x, *d: x.transpose(*d))(kf_f, 1, 2, 0)
        y_f = kv_f * kf_f[None, :, :, :]
        y = (lambda x, s, axes=(-2,-1): jnp.fft.irfft2(x, s=s, axes=axes).astype(jnp.bfloat16))(y_f, (1, L), axes=(1, 2))[:, 0, :S, :]
        y = y + kv * ssm_D[None, None, :]
        return q * y

    a = _A_ref(A_x, A_wqkv, A_wo)
    b = _B_ref(B_q, B_k, B_v, B_shift_k, B_ssm_k, B_ssm_D)
    return jnp.concatenate([a, b], axis=-1)
```

```python
import functools
import numpy as np
import jax
import jax.numpy as jnp
from jax import lax
from jax.experimental import pallas as pl
from jax.experimental.pallas import tpu as pltpu

S = 2048
D = 1024
DH = 32
T = 128
NB = S // T
NG = D // 128
KS = 4
HALO = 16
F32 = jnp.float32
BF16 = jnp.bfloat16


def _consts():
    ang = 2.0 * np.pi * np.outer(np.arange(T) + 0.25, np.arange(T)) / T
    fwd = np.stack([np.cos(ang).reshape(T // 8, 8, T), np.sin(ang).reshape(T // 8, 8, T)], axis=1)
    fwd = fwd.reshape(2 * T, T)
    inv = fwd.T / T
    lane = np.arange(128) // DH
    head_mask = (lane[:, None] == lane[None, :]).astype(np.float32)
    return fwd.astype(np.float32), inv.astype(np.float32), head_mask


def _phi(t):
    return jnp.where(t > 0, t + 1.0, jnp.exp(t)) + 1e-6


def _recip(d):
    r = pl.reciprocal(d, approx=True)
    return r * (2.0 - d * r)


def _dot(a, b):
    return jnp.dot(a, b, preferred_element_type=F32)


class _No:
    def start(self): pass
    def wait(self): pass


def make(unroll=1, dma=True, periods=range(8), flags=None, rep={}, tie=True, MC=256, lag=3):
    def kernel(x_h, wqkv_h, wo_h, q_h, k_h, v_h, sk_h, ssm_h, d_h, fwd_h, inv_h, msk_h, out_h,
               x_v, w_v, wo_v, q_v, k_v, v_v, sk_v, ssm_v, d_v, fwd_v, inv_v, msk_v,
               pkt_v, p_v, z_v, wqt_v, zc_v, pqn_v, m_v, oa_v, ob_v, sems, *rest):
        kv_v, xs_v, ks_v, zs_v = rest[0:3], rest[3:5], rest[5:7], rest[7:9]
        sem_ids = {}

        def copy(name, src, dst):
            if not dma:
                return _No()
            if name not in sem_ids:
                sem_ids[name] = len(sem_ids)
            return pltpu.make_async_copy(src, dst, sems.at[sem_ids[name]])

        HS = S // 2
        cols = lambda g: pl.ds(g * 128, 128)
        cp_x = [copy(("x", h), x_h.at[pl.ds(h * HS, HS)], x_v.at[pl.ds(h * HS, HS)]) for h in range(2)]
        cp_w = [copy(("w", j), wqkv_h.at[:, pl.ds(j * D, D)], w_v.at[:, pl.ds(j * D, D)]) for j in range(3)]
        cp_wo = copy("wo", wo_h, wo_v)
        cp_q = [copy(("q", g), q_h.at[:, cols(g)], q_v.at[g]) for g in range(NG)]
        cp_k = [copy(("k", g), k_h.at[:, cols(g)], k_v.at[g, pl.ds(HALO, S)]) for g in range(NG)]
        cp_v = [copy(("v", g), v_h.at[:, cols(g)], v_v.at[g]) for g in range(NG)]
        cp_s = [copy(("s", g), ssm_h.at[cols(g)], ssm_v.at[g]) for g in range(NG)]
        cp_small = [copy("sk", sk_h, sk_v), copy("d", d_h, d_v), copy("fwd", fwd_h, fwd_v),
                    copy("inv", inv_h, inv_v), copy("msk", msk_h, msk_v)]
        cp_ob = [copy(("ob", g), ob_v.at[g], out_h.at[:, pl.ds(D + g * 128, 128)]) for g in range(NG)]
        cp_oa = [copy(("oa", h), oa_v.at[pl.ds(h * HS, HS)], out_h.at[pl.ds(h * HS, HS), pl.ds(0, D)])
                 for h in range(2)]

        class Plan:
            def __init__(self, nslots):
                self.keep = msk_v[0:8, :].astype(F32) > -1.0
                self.load = [0.0] * nslots
                self.items = [[] for _ in range(nslots)]
                self.pos = 0

            def put(self, slot, cost, fn):
                slot = min(slot, len(self.load) - 1)
                self.load[slot] += cost
                self.items[slot].append(fn)

            def spread(self, lo, hi, items):
                for n, (cost, fn) in enumerate(items):
                    self.put(lo + (n * (hi - lo)) // len(items), cost, fn)

            def fill(self, lo, hi, items):
                total = sum(c for c, _ in items)
                level = (total + sum(self.load[lo:hi])) / (hi - lo)
                while sum(max(level - l, 0.0) for l in self.load[lo:hi]) > total:
                    level -= 0.25
                slot, room = lo, 0.0
                room = max(level - self.load[lo], 0.0)
                for cost, fn in items:
                    while room < cost / 2 and slot < hi - 1:
                        slot += 1
                        room += max(level - self.load[slot], 0.0)
                    room -= cost
                    self.put(slot, cost, fn)

            def slab(self, val):
                toks = []
                for fn in self.items[self.pos]:
                    toks += fn()
                self.pos += 1
                if not toks or not tie:
                    return val
                out = pltpu.bitcast(val, jnp.uint32)
                for tk in toks:
                    tk = pltpu.bitcast(tk, jnp.uint32)
                    for r in range(0, tk.shape[0], 8):
                        out = jnp.where(self.keep, out, tk[r:r + 8])
                return pltpu.bitcast(out, BF16)

            def lhs(self, val):
                m, k = val.shape
                parts = []
                for c in range(0, k, 512):
                    parts.append(jnp.concatenate(
                        [self.slab(val[r:r + 16, c:c + 128]) for r in range(0, m, 16)], axis=0))
                    if min(c + 512, k) > c + 128:
                        parts.append(val[:, c + 128:min(c + 512, k)])
                return parts[0] if len(parts) == 1 else jnp.concatenate(parts, axis=1)

            def finish(self):
                assert self.pos == len(self.load) - 1, (self.pos, len(self.load))
                for fn in self.items[self.pos]:
                    fn()

        def pre_items(g, it, kvs):
            w = sk_v[:, cols(g)].astype(F32)
            wt = [jnp.broadcast_to(w[tau:tau + 1], (16, 128)) for tau in range(KS)]

            def item(n):
                def fn():
                    r0 = pl.multiple_of(it * 2 * T + n * 16, 16)
                    kk = k_v[g, pl.ds(r0, 16 + HALO), :].astype(F32)
                    ksh = kk[HALO:] * wt[0]
                    for tau in range(1, KS):
                        ksh = ksh + kk[HALO - tau:HALO - tau + 16] * wt[tau]
                    kv = (ksh * v_v[g, pl.ds(r0, 16), :].astype(F32)).astype(BF16)
                    kv_v[g % 3][pl.ds(r0, 16), :] = kv
                    kvs.append(kv)
                    return [kv]
                return (36, fn)
            return [item(n) for n in range(2 * T // 16)]

        def fwd_dots(g, it, kvs, plan):
            f = fwd_v[...]
            for b in range(2):
                flt = ssm_v[g, :, pl.ds(pl.multiple_of((it * 2 + b) * T, T), T)]
                ks_v[g % 2][it * 2 + b] = lax.dot_general(
                    plan.lhs(f) if b == 0 else f, flt, (((1,), (1,)), ((), ())), preferred_element_type=F32)
            for b in range(2):
                xs_v[g % 2][it * 2 + b] = _dot(f, jnp.concatenate(kvs[b * 8:(b + 1) * 8], axis=0))

        def mac_items(g, it):
            s = g % 2
            items = []
            for pp in range(2):
                st = dict(res=[[], [], []])
                for part in range(3):
                    for i in range(NB):
                        def fn(pp=pp, part=part, i=i, st=st):
                            r0 = pl.multiple_of((it * 2 + pp) * 16, 16)
                            re, im = pl.ds(r0, 8), pl.ds(r0 + 8, 8)
                            if i == 0:
                                st['x'], st['k'] = [], []
                            if part < 2:
                                st['x'].append(xs_v[s][i, (re, im)[part], :])
                                st['k'].append(ks_v[s][i, (re, im)[part], :])
                            else:
                                st['x'].append(xs_v[s][i, re, :] + xs_v[s][i, im, :])
                                st['k'].append(ks_v[s][i, re, :] + ks_v[s][i, im, :])
                            acc = st['k'][i] * st['x'][0]
                            for j in range(1, i + 1):
                                acc = acc + st['k'][i - j] * st['x'][j]
                            if part < 2:
                                st['res'][part].append(acc)
                                return [acc]
                            p1, p2 = st['res'][0][i], st['res'][1][i]
                            yr, yi = p1 - p2, acc - (p1 + p2)
                            zr = yr if i == 0 else yr + st['yi']
                            zi = yi if i == 0 else yi - st['yr']
                            st['yr'], st['yi'] = yr, yi
                            zz = jnp.concatenate([zr, zi], axis=0).astype(BF16)
                            zs_v[s][i, pl.ds(r0, 16), :] = zz
                            return [zz]
                        items.append((2 * i + 2 + (8 if part == 2 else 0), fn))
            return items

        def inv_dots(g, it, plan):
            gm = inv_v[...]
            return [_dot(plan.lhs(gm) if b == 0 else gm, zs_v[g % 2][it * 2 + b]) for b in range(2)]

        def inv_items(g, it, ys):
            dd = jnp.broadcast_to(d_v[:, cols(g)].astype(F32), (16, 128))

            def item(n):
                def fn():
                    rows = pl.ds(pl.multiple_of(it * 2 * T + n * 16, 16), 16)
                    y = ys[n // 8][(n % 8) * 16:(n % 8 + 1) * 16]
                    y = y + kv_v[g % 3][rows, :].astype(F32) * dd
                    ob = (q_v[g, rows, :].astype(F32) * y).astype(BF16)
                    ob_v[g, rows, :] = ob
                    return [ob]
                return (14, fn)
            return [item(n) for n in range(2 * T // 16)]

        def lanes(it, base=0):
            return pl.ds(pl.multiple_of(base + it * 128, 128), 128)

        def a_k(h, it, c, plan, st):
            rows = pl.ds(h * HS + c * MC, MC)
            res = _dot(plan.lhs(x_v[rows, :]), w_v[:, lanes(it, D)])
            pks = []

            def item(n):
                def fn():
                    pk = _phi(res[n * 16:(n + 1) * 16])
                    part = pk[0:8] + pk[8:16]
                    st['z'] = part if 'z' not in st else st['z'] + part
                    pks.append(pk.astype(BF16))
                    if n % 8 < 7:
                        return [pks[-1]]
                    pkt = jnp.concatenate(pks[-8:], axis=0).T
                    pkt_v[lanes(it), pl.ds(h * HS + c * MC + (n // 8) * 128, 128)] = pkt
                    if c == HS // MC - 1 and n == MC // 16 - 1:
                        z_v[it] = st['z'] if h == 0 else z_v[it] + st['z']
                    return [pks[-1]]
                return (20, fn)
            return [item(n) for n in range(MC // 16)]

        def a_p(h, it, c, plan, st):
            r0 = h * (D // 2) + c * (MC // 2)
            res = _dot(plan.lhs(pkt_v[pl.ds(r0, MC // 2), :]), x_v[:, lanes(it)])

            def item(n):
                def fn():
                    pb = res[n * 16:(n + 1) * 16].astype(BF16)
                    p_v[pl.ds(r0 + n * 16, 16), lanes(it)] = pb
                    return [pb]
                return (2, fn)
            return [item(n) for n in range(MC // 32)]

        def prep_items(h, it):
            def wq(n):
                def fn():
                    r0 = h * (D // 2) + n * 128
                    blk = w_v[pl.ds(r0, 128), lanes(it)].T
                    wqt_v[lanes(it), pl.ds(r0, 128)] = blk
                    return [blk[112:128]]
                return (4, fn)

            def zc():
                z = jnp.sum(z_v[it], axis=0, keepdims=True)
                col = jnp.broadcast_to(z, (128, 128)).T
                zc_v[lanes(it), :] = col
                return [col[120:128]]
            return [wq(n) for n in range(4)] + ([(8, zc)] if h == 1 else [])

        def a_q(h, it, c, plan, st):
            rows = pl.ds(pl.multiple_of(h * HS + it * 128, 128), 128)
            res = lax.dot_general(plan.lhs(wqt_v[pl.ds(c * MC, MC), :]), x_v[rows, :],
                                  (((1,), (1,)), ((), ())), preferred_element_type=F32)
            outs = []

            def item(n):
                def fn():
                    pq = _phi(res[n * DH:(n + 1) * DH])
                    pz = pq * zc_v[pl.ds(c * MC + n * DH, DH), :]
                    den = (pz[0:8] + pz[8:16]) + (pz[16:24] + pz[24:32])
                    for sh in (4, 2, 1):
                        den = den + pltpu.roll(den, sh, 0)
                    inv = _recip(den + 1e-6)
                    outs.append((pq * jnp.concatenate([inv] * 4, axis=0)).astype(BF16))
                    if n % 4 == 3:
                        pqn_v[rows, pl.ds(c * MC + (n // 4) * 128, 128)] = jnp.concatenate(outs[-4:], axis=0).T
                    return [outs[-1]]
                return (56, fn)
            return [item(n) for n in range(MC // DH)]

        def a_o(h, it, c, plan, st):
            r0 = h * HS + c * MC
            res = _dot(plan.lhs(pqn_v[pl.ds(r0, MC), :]), m_v[:, lanes(it)])

            def item(n):
                def fn():
                    ob = res[n * 16:(n + 1) * 16].astype(BF16)
                    oa_v[pl.ds(r0 + n * 16, 16), lanes(it)] = ob
                    return [ob]
                return (2, fn)
            return [item(n) for n in range(MC // 16)]

        def step(p, it):
            has_a = 0 <= p < 8
            has_f, has_m, has_i = p + 1 < NG, 0 <= p < NG, 1 <= p
            nc = HS // MC
            cs = MC // 8
            seq = []
            if p == 4:
                seq.append(('kv', 16))
            for c in range(nc if has_a else 0):
                seq.append((c, cs))
                if c == 0 and has_i:
                    seq.append(('inv', 8))
            if not has_a and has_i:
                seq.append(('inv', 8))
            if p == 4:
                seq.append(('m', 16))
            if has_f:
                seq.append(('fwd', 16))
            start, n = {}, 0
            for name, cnt in seq:
                start[name] = n
                n += cnt
            plan = Plan(n + 1)
            kvs, st = [], {}
            late = {}
            for idx, (name, cnt) in enumerate(seq):
                lo = start[name] + cnt + lag
                if name == 'inv':
                    late[name] = (min(lo, n), min(lo + 32, n + 1), 14 * 16)
                elif isinstance(name, int):
                    late[name] = (min(lo, n), min(lo + cs, n + 1), [20, 1, 28, 2][p // 2] * MC // 16)
            for lo, hi, cost in late.values():
                for sl in range(lo, hi):
                    plan.load[min(sl, n)] += cost / (hi - lo)
            if has_f:
                plan.spread(0, max(start['fwd'] - 8, 1), pre_items(p + 1, it, kvs))
            if p in (2, 3):
                plan.spread(8, n - 8, prep_items(p % 2, it))
            if has_m:
                plan.fill(0, n, mac_items(p, it))

            def place(name, items):
                lo, hi, cost = late[name]
                for sl in range(lo, hi):
                    plan.load[min(sl, n)] -= cost / (hi - lo)
                plan.spread(lo, hi, items)

            for name, cnt in seq:
                if name == 'kv':
                    kvh = _dot(plan.lhs(p_v[lanes(it), :]), w_v[:, lanes(it, 2 * D)])
                    kvh = jnp.where(msk_v[...] > 0, kvh, 0.0).astype(BF16)
                elif name == 'm':
                    mm = _dot(plan.lhs(kvh), wo_v[lanes(it), 0:D // 2])
                    m_v[lanes(it), 0:D // 2] = mm.astype(BF16)
                    mm = _dot(plan.lhs(kvh), wo_v[lanes(it), D // 2:D])
                    m_v[lanes(it), D // 2:D] = mm.astype(BF16)
                elif name == 'inv':
                    place(name, inv_items(p - 1, it, inv_dots(p - 1, it, plan)))
                elif name == 'fwd':
                    fwd_dots(p + 1, it, kvs, plan)
                else:
                    place(name, [a_k, a_p, a_q, a_o][p // 2](p % 2, it, name, plan, st))
            plan.finish()

        def loop(p):
            def body(it, c):
                step(p, it % 8 if p in rep else it)
                return c
            lax.fori_loop(0, 8 * rep.get(p, 1), body, 0, unroll=unroll)

        for c in cp_small:
            c.start()
        cp_k[0].start(); cp_v[0].start(); cp_s[0].start()
        cp_x[0].start(); cp_w[1].start()
        for g in range(NG):
            k_v[g, pl.ds(0, HALO), :] = jnp.zeros((HALO, 128), BF16)
        for c in cp_small:
            c.wait()
        cp_k[0].wait(); cp_v[0].wait(); cp_s[0].wait()
        cp_k[1].start(); cp_v[1].start(); cp_s[1].start()
        loop(-1)
        cp_x[0].wait(); cp_w[1].wait()

        for p in periods:
            if p + 2 < NG:
                cp_k[p + 2].start(); cp_v[p + 2].start(); cp_s[p + 2].start()
            cp_q[p].start()
            if p == 0:
                cp_x[1].start()
            if p == 1:
                cp_x[1].wait(); cp_w[0].start()
            if p == 2:
                cp_w[0].wait(); cp_w[2].start(); cp_wo.start()
            if p == 4:
                cp_w[2].wait(); cp_wo.wait()
            if p + 1 < NG:
                cp_k[p + 1].wait(); cp_v[p + 1].wait(); cp_s[p + 1].wait()
            if p >= 1:
                cp_q[p - 1].wait()

            loop(p)
            if p >= 1:
                cp_ob[p - 1].start()
            if p >= 6:
                cp_oa[p - 6].start()

        cp_q[NG - 1].wait()
        loop(NG)
        cp_ob[NG - 1].start()
        for c in cp_ob + cp_oa:
            c.wait()

    @jax.jit
    def run(A_x, A_wqkv, A_wo, B_q, B_k, B_v, B_shift_k, B_ssm_k, B_ssm_D):
        fwd, inv, msk = _consts()
        any_spec = pl.BlockSpec(memory_space=pl.ANY)
        vm = pltpu.VMEM
        out = pl.pallas_call(
            kernel,
            out_shape=jax.ShapeDtypeStruct((S, 2 * D), BF16),
            in_specs=[any_spec] * 12,
            out_specs=any_spec,
            scratch_shapes=[
                vm((S, D), BF16), vm((D, 3 * D), BF16), vm((D, D), BF16),
                vm((NG, S, 128), BF16), vm((NG, S + HALO, 128), BF16), vm((NG, S, 128), BF16),
                vm((KS, D), BF16), vm((NG, 128, S), BF16), vm((1, D), BF16),
                vm((2 * T, T), BF16), vm((T, 2 * T), BF16), vm((128, 128), BF16),
                vm((D, S), BF16), vm((D, D), BF16), vm((NG, 8, 128), F32), vm((D, D), BF16), vm((D, 128), F32), vm((S, D), BF16),
                vm((D, D), BF16), vm((S, D), BF16), vm((NG, S, 128), BF16),
                pltpu.SemaphoreType.DMA((64,)),
            ] + [vm((S, 128), BF16)] * 3 + [vm((NB, 2 * T, 128), F32)] * 4 + [vm((NB, 2 * T, 128), BF16)] * 2,
            compiler_params=pltpu.CompilerParams(vmem_limit_bytes=100 * 1024 * 1024, flags=flags),
        )(A_x.reshape(S, D), A_wqkv, A_wo, B_q.reshape(S, D), B_k.reshape(S, D), B_v.reshape(S, D),
          B_shift_k.T, B_ssm_k, B_ssm_D.reshape(1, D),
          jnp.asarray(fwd, BF16), jnp.asarray(inv, BF16), jnp.asarray(msk, BF16))
        return out.reshape(1, S, 2 * D)

    return run


pallas_concat_heads__linear_attn_block__ssm_conv_h3__prompt_kernel = make(MC=512)
```

```python
import functools
import numpy as np
import jax
import jax.numpy as jnp
from jax import lax
from jax.experimental import pallas as pl
from jax.experimental.pallas import tpu as pltpu

S = 2048
D = 1024
DH = 32
T = 128
NB = S // T
NG = D // 128
KS = 4
HALO = 16
F32 = jnp.float32
BF16 = jnp.bfloat16


def _consts():
    ang = 2.0 * np.pi * np.outer(np.arange(T) + 0.25, np.arange(T)) / T
    fwd = np.stack([np.cos(ang).reshape(T // 8, 8, T), np.sin(ang).reshape(T // 8, 8, T)], axis=1)
    fwd = fwd.reshape(2 * T, T)
    inv = fwd.T / T
    lane = np.arange(128) // DH
    head_mask = (lane[:, None] == lane[None, :]).astype(np.float32)
    return fwd.astype(np.float32), inv.astype(np.float32), head_mask


def _phi(t):
    return jnp.where(t > 0, t + 1.0, jnp.exp(t)) + 1e-6


def _recip(d):
    r = pl.reciprocal(d, approx=True)
    return r * (2.0 - d * r)


def _aligned(i, n):
    return i if isinstance(i, int) else pl.multiple_of(i, n)


def _dot(a, b):
    return jnp.dot(a, b, preferred_element_type=F32)


class _No:
    def start(self): pass
    def wait(self): pass


def make(unroll=1, dma=True, periods=range(8), flags=None, rep={}, tie=True, MC=512, lag=3, WT=256, all_first=True, tail=(5, 7), orows=((0, 512), (512, 512), (1024, 512), (1536, 256), (1792, 256))):
    def kernel(x_h, wqkv_h, wo_h, q_h, k_h, v_h, sk_h, ssm_h, d_h, fwd_h, inv_h, msk_h, out_h,
               x_v, w_v, wo_v, q_v, k_v, v_v, sk_v, ssm_v, d_v, fwd_v, inv_v, msk_v,
               pkt_v, p_v, z_v, wqt_v, zc_v, pqn_v, m_v, oa_v, ob_v, sems, *rest):
        kv_v, xs_v, ks_v, zs_v = rest[0:3], rest[3:5], rest[5:7], rest[7:9]
        sem_ids = {}

        def copy(name, src, dst):
            if not dma:
                return _No()
            if name not in sem_ids:
                sem_ids[name] = len(sem_ids)
            return pltpu.make_async_copy(src, dst, sems.at[sem_ids[name]])

        cols = lambda g: pl.ds(g * 128, 128)
        XC = 256
        cp_x = [copy(("x", c), x_h.at[pl.ds(c * XC, XC)], x_v.at[pl.ds(c * XC, XC)]) for c in range(S // XC)]
        wcols = [(D + j * WT, WT) for j in range(D // WT)] + [(0, D), (2 * D, D)]
        cp_w = [copy(("w", j), wqkv_h.at[:, pl.ds(c0, n)], w_v.at[:, pl.ds(c0, n)]) for j, (c0, n) in enumerate(wcols)]
        cp_wk, cp_wq, cp_wv = cp_w[:-2], cp_w[-2], cp_w[-1]
        cp_wo = copy("wo", wo_h, wo_v)
        cp_q = [copy(("q", g), q_h.at[:, cols(g)], q_v.at[g]) for g in range(NG)]
        cp_k = [copy(("k", g), k_h.at[:, cols(g)], k_v.at[g, pl.ds(HALO, S)]) for g in range(NG)]
        cp_v = [copy(("v", g), v_h.at[:, cols(g)], v_v.at[g]) for g in range(NG)]
        cp_s = [copy(("s", g), ssm_h.at[cols(g)], ssm_v.at[g]) for g in range(NG)]
        cp_sk, cp_d, cp_fwd = copy("sk", sk_h, sk_v), copy("d", d_h, d_v), copy("fwd", fwd_h, fwd_v)
        cp_inv, cp_msk = copy("inv", inv_h, inv_v), copy("msk", msk_h, msk_v)
        cp_ob = [copy(("ob", g), ob_v.at[g], out_h.at[:, pl.ds(D + g * 128, 128)]) for g in range(NG)]
        cp_oa = [copy(("oa", r0), oa_v.at[pl.ds(r0, n)], out_h.at[pl.ds(r0, n), pl.ds(0, D)]) for r0, n in orows]

        class Plan:
            def __init__(self, nslots):
                self.keep = msk_v[0:8, :].astype(F32) > -1.0
                self.load = [0.0] * nslots
                self.items = [[] for _ in range(nslots)]
                self.pos = 0

            def put(self, slot, cost, fn):
                slot = min(slot, len(self.load) - 1)
                self.load[slot] += cost
                self.items[slot].append(fn)

            def spread(self, lo, hi, items):
                for n, (cost, fn) in enumerate(items):
                    self.put(lo + (n * (hi - lo)) // len(items), cost, fn)

            def fill(self, lo, hi, items):
                total = sum(c for c, _ in items)
                level = (total + sum(self.load[lo:hi])) / (hi - lo)
                while sum(max(level - l, 0.0) for l in self.load[lo:hi]) > total:
                    level -= 0.25
                slot, room = lo, 0.0
                room = max(level - self.load[lo], 0.0)
                for cost, fn in items:
                    while room < cost / 2 and slot < hi - 1:
                        slot += 1
                        room += max(level - self.load[slot], 0.0)
                    room -= cost
                    self.put(slot, cost, fn)

            def slab(self, val):
                toks = []
                for fn in self.items[self.pos]:
                    toks += fn()
                self.pos += 1
                if not toks or not tie:
                    return val
                out = pltpu.bitcast(val, jnp.uint32)
                for tk in toks:
                    tk = pltpu.bitcast(tk, jnp.uint32)
                    for r in range(0, tk.shape[0], 8):
                        out = jnp.where(self.keep, out, tk[r:r + 8])
                return pltpu.bitcast(out, BF16)

            def lhs(self, val):
                m, k = val.shape
                parts = []
                for c in range(0, k, 512):
                    parts.append(jnp.concatenate(
                        [self.slab(val[r:r + 16, c:c + 128]) for r in range(0, m, 16)], axis=0))
                    if min(c + 512, k) > c + 128:
                        parts.append(val[:, c + 128:min(c + 512, k)])
                return parts[0] if len(parts) == 1 else jnp.concatenate(parts, axis=1)

            def finish(self):
                assert self.pos == len(self.load) - 1, (self.pos, len(self.load))
                for fn in self.items[self.pos]:
                    fn()

        def pre_items(g, it, kvs):
            w = sk_v[:, cols(g)].astype(F32)
            wt = [jnp.broadcast_to(w[tau:tau + 1], (16, 128)) for tau in range(KS)]

            def item(n):
                def fn():
                    r0 = _aligned(it * 2 * T + n * 16, 16)
                    kk = k_v[g, pl.ds(r0, 16 + HALO), :].astype(F32)
                    ksh = kk[HALO:] * wt[0]
                    for tau in range(1, KS):
                        ksh = ksh + kk[HALO - tau:HALO - tau + 16] * wt[tau]
                    kv = (ksh * v_v[g, pl.ds(r0, 16), :].astype(F32)).astype(BF16)
                    kv_v[g % 3][pl.ds(r0, 16), :] = kv
                    kvs.append(kv)
                    return [kv]
                return (36, fn)
            return [item(n) for n in range(2 * T // 16)]

        def fwd_filter(g, it, plan):
            f = fwd_v[...]
            for b in range(it * 4, it * 4 + 4):
                ks_v[g % 2][b] = lax.dot_general(
                    plan.lhs(f) if b % 4 == 0 else f, ssm_v[g, :, pl.ds(b * T, T)],
                    (((1,), (1,)), ((), ())), preferred_element_type=F32)

        def fwd_data(g, it, kvs, plan):
            f = fwd_v[...]
            for b in range(4):
                xs_v[g % 2][it * 4 + b] = _dot(plan.lhs(f) if b == 0 else f,
                                               jnp.concatenate(kvs[b * 8:(b + 1) * 8], axis=0))

        def mac_items(g, it):
            s = g % 2
            items = []
            for pp in range(2):
                st = dict(res=[[], [], []])
                for part in range(3):
                    for i in range(NB):
                        def fn(pp=pp, part=part, i=i, st=st):
                            r0 = _aligned((it * 2 + pp) * 16, 16)
                            re, im = pl.ds(r0, 8), pl.ds(r0 + 8, 8)
                            if i == 0:
                                st['x'], st['k'] = [], []
                            if part < 2:
                                st['x'].append(xs_v[s][i, (re, im)[part], :])
                                st['k'].append(ks_v[s][i, (re, im)[part], :])
                            else:
                                st['x'].append(xs_v[s][i, re, :] + xs_v[s][i, im, :])
                                st['k'].append(ks_v[s][i, re, :] + ks_v[s][i, im, :])
                            acc = st['k'][i] * st['x'][0]
                            for j in range(1, i + 1):
                                acc = acc + st['k'][i - j] * st['x'][j]
                            if part < 2:
                                st['res'][part].append(acc)
                                return [acc]
                            p1, p2 = st['res'][0][i], st['res'][1][i]
                            yr, yi = p1 - p2, acc - (p1 + p2)
                            zr = yr if i == 0 else yr + st['yi']
                            zi = yi if i == 0 else yi - st['yr']
                            st['yr'], st['yi'] = yr, yi
                            zz = jnp.concatenate([zr, zi], axis=0).astype(BF16)
                            zs_v[s][i, pl.ds(r0, 16), :] = zz
                            return [zz]
                        items.append((2 * i + 2 + (8 if part == 2 else 0), fn))
            return items

        def inv_dots(g, it, plan):
            gm = inv_v[...]
            return [_dot(plan.lhs(gm) if b == 0 else gm, zs_v[g % 2][it * 2 + b]) for b in range(2)]

        def inv_items(g, it, ys):
            dd = jnp.broadcast_to(d_v[:, cols(g)].astype(F32), (16, 128))

            def item(n):
                def fn():
                    rows = pl.ds(_aligned(it * 2 * T + n * 16, 16), 16)
                    y = ys[n // 8][(n % 8) * 16:(n % 8 + 1) * 16]
                    y = y + kv_v[g % 3][rows, :].astype(F32) * dd
                    ob = (q_v[g, rows, :].astype(F32) * y).astype(BF16)
                    ob_v[g, rows, :] = ob
                    return [ob]
                return (14, fn)
            return [item(n) for n in range(2 * T // 16)]

        def lanes(it, base=0):
            return pl.ds(base + it * 128, 128)

        def a_k(r0, mc, it, plan):
            st = {}
            rows = pl.ds(r0, mc)
            res = _dot(plan.lhs(x_v[rows, :]), w_v[:, lanes(it, D)])
            pks = []

            def item(n):
                def fn():
                    pk = _phi(res[n * 16:(n + 1) * 16])
                    part = pk[0:8] + pk[8:16]
                    st['z'] = part if 'z' not in st else st['z'] + part
                    pks.append(pk.astype(BF16))
                    if n % 8 < 7:
                        return [pks[-1]]
                    pkt = jnp.concatenate(pks[-8:], axis=0).T
                    pkt_v[lanes(it), pl.ds(r0 + (n // 8) * 128, 128)] = pkt
                    if n == mc // 16 - 1:
                        z_v[it] = st['z'] if r0 == 0 else z_v[it] + st['z']
                    return [pks[-1]]
                return (20, fn)
            return [item(n) for n in range(mc // 16)]

        def a_p(r0, mc, it, plan):
            r0, mc = r0 // 2, mc // 2
            res = _dot(plan.lhs(pkt_v[pl.ds(r0, mc), :]), x_v[:, lanes(it)])

            def item(n):
                def fn():
                    pb = res[n * 16:(n + 1) * 16].astype(BF16)
                    p_v[pl.ds(r0 + n * 16, 16), lanes(it)] = pb
                    return [pb]
                return (2, fn)
            return [item(n) for n in range(mc // 16)]

        def prep_items(h, it):
            def wq(n):
                def fn():
                    r0 = h * (D // 2) + n * 128
                    blk = w_v[pl.ds(r0, 128), lanes(it)].T
                    wqt_v[lanes(it), pl.ds(r0, 128)] = blk
                    return [blk[112:128]]
                return (4, fn)

            def zc():
                z = jnp.sum(z_v[it], axis=0, keepdims=True)
                col = jnp.broadcast_to(z, (128, 128)).T
                zc_v[lanes(it), :] = col
                return [col[120:128]]
            return [wq(n) for n in range(4)] + ([(8, zc)] if h == 1 else [])

        def a_q(f0, mc, it, plan):
            rows = pl.ds(it * 128, 128)
            res = lax.dot_general(plan.lhs(wqt_v[pl.ds(f0, mc), :]), x_v[rows, :],
                                  (((1,), (1,)), ((), ())), preferred_element_type=F32)
            outs = []

            def item(n):
                def fn():
                    pq = _phi(res[n * DH:(n + 1) * DH])
                    pz = pq * zc_v[pl.ds(f0 + n * DH, DH), :]
                    den = (pz[0:8] + pz[8:16]) + (pz[16:24] + pz[24:32])
                    for sh in (4, 2, 1):
                        den = den + pltpu.roll(den, sh, 0)
                    inv = _recip(den + 1e-6)
                    outs.append((pq * jnp.concatenate([inv] * 4, axis=0)).astype(BF16))
                    if n % 4 == 3:
                        pqn_v[rows, pl.ds(f0 + (n // 4) * 128, 128)] = jnp.concatenate(outs[-4:], axis=0).T
                    return [outs[-1]]
                return (56, fn)
            return [item(n) for n in range(mc // DH)]

        def a_o(r0, mc, it, plan):
            res = _dot(plan.lhs(pqn_v[pl.ds(r0, mc), :]), m_v[:, lanes(it)])

            def item(n):
                def fn():
                    ob = res[n * 16:(n + 1) * 16].astype(BF16)
                    oa_v[pl.ds(r0 + n * 16, 16), lanes(it)] = ob
                    return [ob]
                return (2, fn)
            return [item(n) for n in range(mc // 16)]

        a_fn = dict(k=a_k, p=a_p, q=a_q, o=a_o)
        a_cost = dict(k=20 / 16, p=1 / 16, q=28 / 16, o=2 / 16)

        def block(work, vec):
            work = sorted(work, key=lambda e: e[0])
            seq = [e for _, e in work]
            start, n = [], 0
            for e in seq:
                start.append(n)
                n += e[2] // 8 if e[0] in a_fn else dict(kv=16, m=16, inv=8, ff=16, fd=16, dma=0)[e[0]]
            start.append(n)
            slot_at = lambda t: start[sum(1 for tt, _ in work if tt < t)]
            plan = Plan(n + 1)
            late, kvs, prev = {}, {}, 0
            for i, e in enumerate(seq):
                lo = min(start[i + 1] + lag, n)
                if e[0] == 'inv':
                    late[i] = (lo, min(lo + 24, n + 1), 14 * 16)
                elif e[0] in a_fn:
                    late[i] = (lo, min(lo + e[2] // 8, n + 1), a_cost[e[0]] * e[2])
                elif e[0] == 'fd':
                    kvs[i] = []
                    lo = max(prev, start[i] - 160)
                    plan.spread(lo, max(start[i] - 8, lo + 1),
                                pre_items(e[1], 2 * e[2], kvs[i]) + pre_items(e[1], 2 * e[2] + 1, kvs[i]))
                    prev = start[i]
            for lo, hi, cost in late.values():
                for sl in range(lo, hi):
                    plan.load[sl] += cost / (hi - lo)
            for items, first, last, even in vec:
                (plan.spread if even else plan.fill)(slot_at(first), max(slot_at(last), slot_at(first) + 1), items)
            done = [0]

            def place(i, items):
                lo, hi, cost = late[i]
                for sl in range(lo, hi):
                    plan.load[sl] -= cost / (hi - lo)
                plan.spread(lo, hi, items)
                done[0] = max(done[0], hi - 1)

            for i, e in enumerate(seq):
                if e[0] == 'kv':
                    kvh = _dot(plan.lhs(p_v[lanes(e[1]), :]), w_v[:, lanes(e[1], 2 * D)])
                    kvh = jnp.where(msk_v[...] > 0, kvh, 0.0).astype(BF16)
                elif e[0] == 'm':
                    for c in range(2):
                        half = pl.ds(c * (D // 2), D // 2)
                        m_v[lanes(e[1]), half] = _dot(plan.lhs(kvh), wo_v[lanes(e[1]), half]).astype(BF16)
                elif e[0] == 'inv':
                    place(i, inv_items(e[1], e[2], inv_dots(e[1], e[2], plan)))
                elif e[0] == 'ff':
                    fwd_filter(e[1], e[2], plan)
                elif e[0] == 'fd':
                    fwd_data(e[1], e[2], kvs[i], plan)
                elif e[0] == 'dma':
                    plan.put(max(done[0], plan.pos), 0, lambda c=e[1]: (c.start(), [])[1])
                else:
                    place(i, a_fn[e[0]](e[1], e[2], e[3], plan))
            plan.finish()

        def a_work(p):
            h = p % 2
            if p in (4, 5):
                res = [(u + c * MC / D, ('q', c * MC, MC, h * 8 + u)) for u in range(8) for c in range(D // MC)]
                for g in range(h * 4, h * 4 + 4):
                    res += [(2 * (g % 4) + 0.3, ('kv', g)), (2 * (g % 4) + 1.3, ('m', g))]
                return res
            if p >= 6:
                res = []
                for (r0, n), cp in zip(orows, cp_oa):
                    if r0 // D == h:
                        t0 = (r0 % D) / 128
                        res += [(t0 + it * n / D, ('o', r0, n, it)) for it in range(8)]
                        res.append((t0 + 7.5 * n / D, ('dma', cp)))
                return res
            mc = XC if p == 0 else MC
            return [((c * 8 + it) * mc / D, ('kp'[p // 2], h * D + c * mc, mc, it))
                    for c in range(D // mc) for it in range(8)]

        def spread(t0, t1, es):
            return [(t0 + (n + 0.5) * (t1 - t0) / len(es), e) for n, e in enumerate(es)]

        def fwd_work(g):
            return [(kind, g, it) for it in range(4) for kind in ('ff', 'fd')]

        def all_macs(g):
            return sum([mac_items(g, it) for it in range(8)], [])

        grp = lambda g: [cp_s[g], cp_k[g], cp_v[g]]
        first = [cp_fwd, cp_msk, cp_s[0]]
        order0 = first + [cp_sk, cp_k[0], cp_v[0], cp_x[0]] + cp_wk + [cp_x[1]] + grp(1) + [cp_x[2], cp_x[3]]
        order1 = [cp_inv, cp_d, cp_q[0]] + grp(2) + cp_x[4:]
        order2 = [cp_q[1], cp_wq] + grp(3)
        order3 = cp_q[2:] + sum([grp(g) for g in range(4, NG)], []) + [cp_wv, cp_wo]
        for c in order0 + (order1 + order2 + order3 if all_first else []):
            c.start()
        for g in range(NG):
            k_v[g, pl.ds(0, HALO), :] = jnp.zeros((HALO, 128), BF16)

        def wait(cs):
            for c in cs:
                c.wait()

        wait(first)
        block(spread(0, 1, [('ff', 0, it) for it in range(4)]), [])
        wait([cp_sk, cp_k[0], cp_v[0]])
        block(spread(0, 1, [('fd', 0, it) for it in range(4)]), [])

        work = a_work(0) + spread(4, 8, fwd_work(1))
        macs = all_macs(0)
        nw = len(cp_wk)
        cuts = [2 * j / nw for j in range(nw + 1)] + [4, 8]
        needs = [[cp_x[0], cp_wk[0]]] + [[c] for c in cp_wk[1:]] + [[cp_x[1]], grp(1) + [cp_x[2], cp_x[3]]]
        for j, need in enumerate(needs):
            wait(need)
            if j == nw and not all_first:
                for c in order1 + order2:
                    c.start()
            t0, t1 = cuts[j], cuts[j + 1]
            block([e for e in work if t0 <= e[0] < t1],
                  [(macs[int(len(macs) * t0 / 8):int(len(macs) * t1 / 8)], t0, t1, False)])

        for p in range(1, 8):
            if p == 1:
                wait(order1)
                if not all_first:
                    for c in order3:
                        c.start()
            if p == 2:
                wait(order2)
            if p == 3:
                wait(order3)
            work, vec = a_work(p), []
            if p < 7:
                work += spread(0, 8, fwd_work(p + 1))
                work += spread(0.2, 8.2 - 0.6, [('inv', p - 1, it) for it in range(8)] + [('dma', cp_ob[p - 1])])
                mac_end = 8
            else:
                work += spread(0, 4, [('inv', 6, it) for it in range(8)] + [('dma', cp_ob[6])])
                work += spread(tail[0] + 0.1, tail[1], [('inv', 7, it) for it in range(8)] + [('dma', cp_ob[7])])
                mac_end = tail[0]
            if p in (2, 3):
                vec.append((sum([prep_items(p % 2, it) for it in range(8)], []), 0.2, 7.8, True))
            vec.append((all_macs(p), 0, mac_end, False))
            block(work, vec)
        wait(cp_ob + cp_oa)

    @jax.jit
    def run(A_x, A_wqkv, A_wo, B_q, B_k, B_v, B_shift_k, B_ssm_k, B_ssm_D):
        fwd, inv, msk = _consts()
        any_spec = pl.BlockSpec(memory_space=pl.ANY)
        vm = pltpu.VMEM
        out = pl.pallas_call(
            kernel,
            out_shape=jax.ShapeDtypeStruct((S, 2 * D), BF16),
            in_specs=[any_spec] * 12,
            out_specs=any_spec,
            scratch_shapes=[
                vm((S, D), BF16), vm((D, 3 * D), BF16), vm((D, D), BF16),
                vm((NG, S, 128), BF16), vm((NG, S + HALO, 128), BF16), vm((NG, S, 128), BF16),
                vm((KS, D), BF16), vm((NG, 128, S), BF16), vm((1, D), BF16),
                vm((2 * T, T), BF16), vm((T, 2 * T), BF16), vm((128, 128), BF16),
                vm((D, S), BF16), vm((D, D), BF16), vm((NG, 8, 128), F32), vm((D, D), BF16), vm((D, 128), F32), vm((S, D), BF16),
                vm((D, D), BF16), vm((S, D), BF16), vm((NG, S, 128), BF16),
                pltpu.SemaphoreType.DMA((64,)),
            ] + [vm((S, 128), BF16)] * 3 + [vm((NB, 2 * T, 128), F32)] * 4 + [vm((NB, 2 * T, 128), BF16)] * 2,
            compiler_params=pltpu.CompilerParams(vmem_limit_bytes=100 * 1024 * 1024, flags=flags),
        )(A_x.reshape(S, D), A_wqkv, A_wo, B_q.reshape(S, D), B_k.reshape(S, D), B_v.reshape(S, D),
          B_shift_k.T, B_ssm_k, B_ssm_D.reshape(1, D),
          jnp.asarray(fwd, BF16), jnp.asarray(inv, BF16), jnp.asarray(msk, BF16))
        return out.reshape(1, S, 2 * D)

    return run


pallas_concat_heads__linear_attn_block__ssm_conv_h3__prompt_kernel = make()
```

```python
import functools
import numpy as np
import jax
import jax.numpy as jnp
from jax import lax
from jax.experimental import pallas as pl
from jax.experimental.pallas import tpu as pltpu

S = 2048
D = 1024
DH = 32
T = 128
NB = S // T
NG = D // 128
KS = 4
HALO = 8
F32 = jnp.float32
BF16 = jnp.bfloat16
U32 = jnp.uint32


def _consts():
    ang = 2.0 * np.pi * np.outer(np.arange(T) + 0.25, np.arange(T)) / T
    fwd = np.stack([np.cos(ang), np.sin(ang)], axis=1)
    fwd = fwd.reshape(2, T // 16, 8, 2, T).transpose(1, 0, 3, 2, 4).reshape(2 * T, T)
    inv = np.stack([np.cos(ang), np.sin(ang)], axis=1)[:T // 2].reshape(T, T).T / T
    inv = np.concatenate([inv[0::2], inv[1::2]], axis=0)
    lane = np.arange(128) // DH
    head_mask = (lane[:, None] == lane[None, :]).astype(np.float32)
    return fwd.astype(np.float32), inv.astype(np.float32), head_mask


def _phi(t):
    return jnp.where(t > 0, t + 1.0, jnp.exp(t)) + 1e-6


def _recip(d):
    r = pl.reciprocal(d, approx=True)
    return r * (2.0 - d * r)


def _aligned(i, n):
    return i if isinstance(i, int) else pl.multiple_of(i, n)


def _pack(x):
    return pltpu.bitcast(x, U32)


def _unpack(x):
    return pltpu.bitcast(x, BF16)


def _split(w):
    return [pltpu.unpack_elementwise(w, index=i, packed_dtype=BF16, unpacked_dtype=F32) for i in range(2)]


def _merge(even, odd):
    return pltpu.pack_elementwise([even, odd], packed_dtype=BF16)


def _dot(a, b):
    return jnp.dot(a, b, preferred_element_type=F32)


class _No:
    def start(self): pass
    def wait(self): pass


def make(unroll=1, dma=True, periods=range(8), flags=None, rep=None, tie=True, MC=1024, lag=3, barrier='sem', nsub=1, scopes=False, gate_every=0, gate_shift=0, tie_st=False, WT=256, depth=20, ahead=8, tail=(5, 7), orows=((0, 1024), (1024, 512), (1536, 256), (1792, 128), (1920, 128))):
    def kernel(x_h, wqkv_h, wo_h, q_h, k_h, v_h, sk_h, ssm_h, d_h, fwd_h, inv_h, msk_h, out_h,
               x_v, w_v, wo_v, q_v, k_v, v_v, sk_v, ssm_v, d_v, fwd_v, inv_v, msk_v,
               fu_v, gu_v, kf_v, pkt_v, p_v, z_v, wqt_v, zc_v, pqn_v, m_v, oa_v, ob_v, sems, bar, *rest):
        kv_v, xs_v, ks_v, zs_v = rest[0:3], rest[3:5], rest[5:7], rest[7:9]
        sem_ids = {}

        def copy(name, src, dst):
            if not dma:
                return _No()
            if name not in sem_ids:
                sem_ids[name] = len(sem_ids)
            return pltpu.make_async_copy(src, dst, sems.at[sem_ids[name]])

        d_row = lambda g: d_v[...].astype(F32)[g * 128:(g + 1) * 128].reshape(1, 128)
        cols = lambda g: pl.ds(g * 128, 128)
        xw_v, ku_v, vu_v, qu_v, obu_v = [r.bitcast(U32) for r in (x_v, k_v, v_v, q_v, ob_v)]
        XC = 256
        cp_x = [[copy(("x", r0, g), x_h.at[pl.ds(r0, n), cols(g)], x_v.at[g, pl.ds(r0, n)]) for g in range(NG)]
                for r0, n in ((0, XC), (XC, XC), (2 * XC, 2 * XC), (4 * XC, S - 4 * XC))]
        wcols = [(D + j * WT, WT) for j in range(D // WT)] + [(0, D), (2 * D, D)]
        cp_w = [copy(("w", j), wqkv_h.at[:, pl.ds(c0, n)], w_v.at[:, pl.ds(c0, n)]) for j, (c0, n) in enumerate(wcols)]
        cp_wk, cp_wq, cp_wv = cp_w[:-2], cp_w[-2], cp_w[-1]
        cp_wo = copy("wo", wo_h, wo_v)
        cp_q = [copy(("q", g), q_h.at[:, cols(g)], q_v.at[g]) for g in range(NG)]
        cp_k = [copy(("k", g), k_h.at[:, cols(g)], k_v.at[g]) for g in range(NG)]
        cp_v = [copy(("v", g), v_h.at[:, cols(g)], v_v.at[g]) for g in range(NG)]
        cp_s = [copy(("s", g), ssm_h.at[cols(g)], ssm_v.at[g]) for g in range(NG)]
        cp_sk, cp_d, cp_fwd = copy("sk", sk_h, sk_v), copy("d", d_h, d_v), copy("fwd", fwd_h, fwd_v)
        cp_inv, cp_msk = copy("inv", inv_h, inv_v), copy("msk", msk_h, msk_v)
        cp_ob = [copy(("ob", g), ob_v.at[g], out_h.at[:, pl.ds(D + g * 128, 128)]) for g in range(NG)]
        cp_oa = [copy(("oa", r0), oa_v.at[pl.ds(r0, n)], out_h.at[pl.ds(r0, n), pl.ds(0, D)]) for r0, n in orows]

        class Plan:
            def __init__(self, nslots):
                self.keep = msk_v[0:8, :].astype(F32) > -1.0
                self.load = [0.0] * nslots
                self.items = [[] for _ in range(nslots)]
                self.pos = 0
                self.prev, self.span, self.gated = None, (0, 1), {}

            def started(self, nslots):
                self.span = (self.pos, nslots)

            def gate(self, ref, *idx):
                if self.prev is None or gate_every == 0 or self.pos - self.gated.get(id(ref), -gate_every) < gate_every:
                    return
                self.gated[id(ref)] = self.pos
                n = self.prev.shape[0] // 8
                r = min(n - 1, max(0, ((self.pos - self.span[0]) * n) // self.span[1] + gate_shift))
                ref[idx + (rows_at(0, 8, self.pos), slice(None))] = pltpu.bitcast(self.prev[r * 8:(r + 1) * 8], ref.dtype)

            def put(self, slot, cost, fn):
                slot = min(slot, len(self.load) - 1)
                self.load[slot] += cost
                self.items[slot].append(fn)

            def spread(self, lo, hi, items):
                for n, (cost, fn) in enumerate(items):
                    self.put(lo + (n * (hi - lo)) // len(items), cost, fn)

            def fill(self, lo, hi, items):
                total = sum(c for c, _ in items)
                level = (total + sum(self.load[lo:hi])) / (hi - lo)
                while sum(max(level - l, 0.0) for l in self.load[lo:hi]) > total:
                    level -= 0.25
                slot, room = lo, 0.0
                room = max(level - self.load[lo], 0.0)
                for cost, fn in items:
                    while room < cost / 2 and slot < hi - 1:
                        slot += 1
                        room += max(level - self.load[slot], 0.0)
                    room -= cost
                    self.put(slot, cost, fn)

            def slab(self, val, step):
                toks = []
                for _ in range(step):
                    for fn in self.items[self.pos]:
                        toks += fn()
                    self.pos += 1
                if not toks or not tie:
                    return val
                for tk in toks:
                    val = jnp.where(self.keep, val, tk if tk.dtype == U32 else pltpu.bitcast(tk, U32))
                return val

            def lhs(self, val, step=1):
                m, k = val.shape
                parts = []
                for c in range(0, k, 512):
                    parts.append(jnp.concatenate(
                        [self.slab(val[r:r + 8, c:c + 128], step) for r in range(0, m, 8)], axis=0))
                    if min(c + 512, k) > c + 128:
                        parts.append(val[:, c + 128:min(c + 512, k)])
                return _unpack(parts[0] if len(parts) == 1 else jnp.concatenate(parts, axis=1))

            def finish(self):
                assert self.pos == len(self.load) - 1, (self.pos, len(self.load))
                for fn in self.items[self.pos]:
                    fn()

        zeros, cur = [], [None]

        def rows_at(r0, n, salt):
            return pl.ds(pl.multiple_of(r0 + zeros[salt % len(zeros)], 8), n)

        def pre_items(g, it, kvs, plan):
            w = sk_v[:, cols(g)].astype(F32)
            w0, w1, w2, w3 = [jnp.broadcast_to(w[tau:tau + 1], (8, 128)) for tau in range(KS)]

            def item(n):
                def fn():
                    r0 = it * T + n * 8
                    for r in range(0 if r0 == 0 else r0 + ahead, min(r0 + ahead + 8, S // 2), 8):
                        for j, kk in enumerate(_split(ku_v[g, pl.ds(r, 8), :])):
                            kf_v[j, pl.ds(HALO + r, 8), :] = kk
                    ve, vo = _split(vu_v[g, pl.ds(r0, 8), :])
                    ke = kf_v[0, pl.ds(HALO + r0, 8), :]
                    ko = kf_v[1, pl.ds(HALO + r0, 8), :]
                    ke1 = kf_v[0, pl.ds(HALO + r0 - 1, 8), :]
                    ko1 = kf_v[1, pl.ds(HALO + r0 - 1, 8), :]
                    ko2 = kf_v[1, pl.ds(HALO + r0 - 2, 8), :]
                    se = (ke * w0 + ko1 * w1) + (ke1 * w2 + ko2 * w3)
                    so = (ko * w0 + ke * w1) + (ko1 * w2 + ke1 * w3)
                    kv = _merge(se * ve, so * vo)
                    kv_v[g % 3][pl.ds(r0, 8), :] = kv
                    kvs.append(kv)
                    return [kv]
                return (22, fn)
            return [item(n) for n in range(2 * T // 16)]

        def fwd_filter(g, it, plan):
            for b in range(it * 4, it * 4 + 4):
                f = fu_v[rows_at(0, T, b), :]
                ks_v[g % 2][b] = lax.dot_general(
                    plan.lhs(f) if b % 4 == 0 else _unpack(f), ssm_v[g, :, pl.ds(b * T, T)],
                    (((1,), (1,)), ((), ())), preferred_element_type=F32)

        def fwd_data(g, it, kvs, plan):
            for b in range(4):
                f = fu_v[rows_at(0, T, it * 4 + b + 8), :]
                xs_v[g % 2][it * 4 + b] = _dot(plan.lhs(f) if b == 0 else _unpack(f),
                                               _unpack(jnp.concatenate(kvs[b * 8:(b + 1) * 8], axis=0)))

        def mac_items(g, it):
            s = g % 2
            items, low = [], []
            for pp in range(2):
                st = dict(res=[[], [], []])
                for part in range(3):
                    for i in range(NB):
                        def fn(pp=pp, part=part, i=i, st=st):
                            r0 = _aligned((it * 2 + pp) * 16, 16)
                            re, im = pl.ds(r0, 8), pl.ds(r0 + 8, 8)
                            if i == 0:
                                st['x'], st['k'] = [], []
                            if part < 2:
                                st['x'].append(xs_v[s][i, (re, im)[part], :])
                                st['k'].append(ks_v[s][i, (re, im)[part], :])
                            else:
                                st['x'].append(xs_v[s][i, re, :] + xs_v[s][i, im, :])
                                st['k'].append(ks_v[s][i, re, :] + ks_v[s][i, im, :])
                            acc = st['k'][i] * st['x'][0]
                            for j in range(1, i + 1):
                                acc = acc + st['k'][i - j] * st['x'][j]
                            if part < 2:
                                st['res'][part].append(acc)
                                return [acc]
                            p1, p2 = st['res'][0][i], st['res'][1][i]
                            yr, yi = p1 - p2, acc - (p1 + p2)
                            zr = yr if i == 0 else yr + st['yi']
                            zi = yi if i == 0 else yi - st['yr']
                            st['yr'], st['yi'] = yr, yi
                            if pp == 0:
                                low.append((zr, zi))
                                return [zr if i % 2 else zi]
                            ar, ai = low[i]
                            ze, zo = _merge(ar + zr, ai + zi), _merge(ar - zr, ai - zi)
                            zs_v[s][i, pl.ds(it * 8, 8), :] = ze
                            zs_v[s][i, pl.ds(T // 2 + it * 8, 8), :] = zo
                            return [zo if i % 2 else ze]
                        items.append((2 * i + 2 + (7 + 6 * pp if part == 2 else 0), fn))
            return items

        def inv_dots(g, it, plan):
            ys = []
            for n in range(8):
                half = (n % 2) * (T // 2)
                gm = gu_v[rows_at(half // 2, T // 4, it * 8 + n), :]
                ys.append(_dot(plan.lhs(gm) if n % 4 == 0 else _unpack(gm),
                               _unpack(zs_v[g % 2][it * 4 + n // 2, pl.ds(half, T // 2), :])))
            return ys

        def inv_items(g, it, ys):
            dd = jnp.broadcast_to(d_row(g), (8, 128))

            def item(n):
                def fn():
                    rows = pl.ds(it * 2 * T + n * 8, 8)
                    ye, yo = [ys[(n // 8) * 2 + j][(n % 8) * 8:(n % 8 + 1) * 8] for j in range(2)]
                    kve, kvo = _split(kv_v[g % 3][rows, :])
                    qe, qo = _split(qu_v[g, rows, :])
                    ob = _merge(qe * (ye + kve * dd), qo * (yo + kvo * dd))
                    obu_v[g, rows, :] = ob
                    return [ob]
                return (12, fn)
            return [item(n) for n in range(4 * T // 16)]

        def lanes(it, base=0):
            return pl.ds(base + it * 128, 128)

        def a_k(r0, mc, it, plan):
            st = {}
            rows = rows_at(r0 // 2, mc // 2, it)
            xu = jnp.concatenate([xw_v[g, rows, :] for g in range(NG)], axis=1)
            res = _dot(plan.lhs(xu), w_v[:, lanes(it, D)])
            pks = []
            plan.prev = res

            def item(n):
                def fn():
                    pk = _phi(res[n * 16:(n + 1) * 16])
                    part = pk[0:8] + pk[8:16]
                    st['z'] = part if 'z' not in st else st['z'] + part
                    pks.append(pk)
                    if n % 8 < 7:
                        return [part]
                    pkt = jnp.concatenate(pks[-8:], axis=0).astype(BF16).T
                    pkt_v[pl.ds(it * 64, 64), pl.ds(r0 + (n // 8) * 128, 128)] = _pack(pkt)
                    if n == mc // 16 - 1:
                        z_v[it] = st['z'] if r0 == 0 else z_v[it] + st['z']
                    return [part]
                return (20, fn)
            return [item(n) for n in range(mc // 16)]

        def a_p(r0, mc, it, plan):
            r0, mc = r0 // 2, mc // 2
            res = _dot(plan.lhs(pkt_v[rows_at(r0 // 2, mc // 2, it), :]), _unpack(xw_v[it, rows_at(0, S // 2, r0 // mc), :]))
            plan.prev = res

            def item(n):
                def fn():
                    pb = _merge(res[n * 16:n * 16 + 8], res[n * 16 + 8:n * 16 + 16])
                    p_v[pl.ds(r0 // 2 + n * 8, 8), lanes(it)] = pb
                    return [pb]
                return (2, fn)
            return [item(n) for n in range(mc // 16)]

        def prep_items(h, it):
            def wq(n):
                def fn():
                    r0 = h * (D // 2) + n * 128
                    blk = _pack(w_v[pl.ds(r0, 128), lanes(it)].T)
                    wqt_v[pl.ds(it * 64, 64), pl.ds(r0, 128)] = blk
                    return [blk[56:64]]
                return (4, fn)

            def zc():
                z = jnp.sum(z_v[it], axis=0, keepdims=True)
                col = jnp.broadcast_to(z, (128, 128)).T
                zc_v[lanes(it), :] = col
                return [col[120:128]]
            return [wq(n) for n in range(4)] + ([(8, zc)] if h == 1 else [])

        def a_q(f0, mc, it, plan):
            rows = pl.ds(it * 64, 64)
            xr = rows_at(it * 64, 64, f0 // mc)
            xu = jnp.concatenate([xw_v[g, xr, :] for g in range(NG)], axis=1)
            res = lax.dot_general(plan.lhs(wqt_v[rows_at(f0 // 2, mc // 2, it), :]), _unpack(xu),
                                  (((1,), (1,)), ((), ())), preferred_element_type=F32)
            outs = []
            plan.prev = res

            def item(n):
                def fn():
                    pq = _phi(res[n * DH:(n + 1) * DH])
                    pz = pq * zc_v[pl.ds(f0 + n * DH, DH), :]
                    den = (pz[0:8] + pz[8:16]) + (pz[16:24] + pz[24:32])
                    for sh in (4, 2, 1):
                        den = den + pltpu.roll(den, sh, 0)
                    inv = _recip(den + 1e-6)
                    pqn = pq * jnp.concatenate([inv] * 4, axis=0)
                    outs.extend([_merge(pqn[0:8], pqn[8:16]), _merge(pqn[16:24], pqn[24:32])])
                    if n % 4 == 3:
                        pqn_v[rows, pl.ds(f0 + (n // 4) * 128, 128)] = _pack(_unpack(jnp.concatenate(outs[-8:], axis=0)).T)
                    return outs[-2:]
                return (56, fn)
            return [item(n) for n in range(mc // DH)]

        def a_o(r0, mc, it, plan):
            res = _dot(plan.lhs(pqn_v[rows_at(r0 // 2, mc // 2, it), :]), m_v[:, lanes(it)])
            plan.prev = res

            def item(n):
                def fn():
                    ob = res[n * 16:(n + 1) * 16].astype(BF16)
                    oa_v[pl.ds(r0 + n * 16, 16), lanes(it)] = ob
                    return [ob[8:16].astype(F32)] if tie_st else []
                return (2, fn)
            return [item(n) for n in range(mc // 16)]

        a_fn = dict(k=a_k, p=a_p, q=a_q, o=a_o)
        a_cost = dict(k=20 / 16, p=1 / 16, q=28 / 16, o=2 / 16)

        nblk = [0]

        def block(work, vec):
            nblk[0] += 1
            if barrier == 'sem':
                pl.semaphore_signal(bar, 1)
                pl.semaphore_wait(bar, 1)
            elif barrier == 'delay':
                pl.delay(1)
            if rep and nblk[0] == rep[0]:
                if 'm' in rep[2]:
                    block_(work, vec)
                    work = [e for e in work if e[1][0] != 'dma']
                    vec = []
                if 'b' in rep[2]:
                    work = [e for e in work if e[1][0] in 'kpqo']
                dmas = [e for e in work if e[1][0] == 'dma']
                work = [e for e in work if e[1][0] != 'dma']
                lax.fori_loop(0, rep[1], lambda i, c: (block_(work, vec), c)[1], 0)
                for e in dmas:
                    e[1][1].start()
                return
            if not scopes:
                return block_(work, vec)
            with jax.named_scope("blk%02d" % nblk[0]):
                block_(work, vec)

        def block_(work, vec):
            work = sorted(work, key=lambda e: e[0])
            seq = [e for _, e in work]
            start, n = [], 0
            for e in seq:
                start.append(n)
                n += e[2] // 8 if e[0] in a_fn else dict(kv=16, m=16, inv=8, ff=16, fd=16, dma=0)[e[0]]
            start.append(n)
            slot_at = lambda t: start[sum(1 for tt, _ in work if tt < t)]
            plan = cur[0] = Plan(n + 1)
            late, kvs, prev = {}, {}, 0
            for i, e in enumerate(seq):
                lo = min(start[i + 1] + lag, n)
                if e[0] == 'inv':
                    late[i] = (lo, min(lo + 48, n + 1), 12 * 32)
                elif e[0] in a_fn:
                    late[i] = (lo, min(lo + e[2] // 8, n + 1), a_cost[e[0]] * e[2])
                elif e[0] == 'fd':
                    kvs[i] = []
                    lo = max(prev, start[i] - 160)
                    plan.spread(lo, max(start[i] - 8, lo + 1),
                                pre_items(e[1], 2 * e[2], kvs[i], plan) + pre_items(e[1], 2 * e[2] + 1, kvs[i], plan))
                    prev = start[i]
            for lo, hi, cost in late.values():
                for sl in range(lo, hi):
                    plan.load[sl] += cost / (hi - lo)
            for items, first, last, even in vec:
                (plan.spread if even else plan.fill)(slot_at(first), max(slot_at(last), slot_at(first) + 1), items)
            done = [0]

            def place(i, items):
                lo, hi, cost = late[i]
                for sl in range(lo, hi):
                    plan.load[sl] -= cost / (hi - lo)
                plan.spread(lo, hi, items)
                done[0] = max(done[0], hi - 1)

            for i, e in enumerate(seq):
                plan.started(max(start[i + 1] - start[i], 1))
                if e[0] == 'kv':
                    kvh = _dot(plan.lhs(p_v[pl.ds(e[1] * 64, 64), :]), w_v[:, lanes(e[1], 2 * D)])
                    kvh = _pack(jnp.where(msk_v[...] > 0, kvh, 0.0).astype(BF16))
                elif e[0] == 'm':
                    for c in range(2):
                        half = pl.ds(c * (D // 2), D // 2)
                        m_v[lanes(e[1]), half] = _dot(plan.lhs(kvh), wo_v[lanes(e[1]), half]).astype(BF16)
                elif e[0] == 'inv':
                    place(i, inv_items(e[1], e[2], inv_dots(e[1], e[2], plan)))
                elif e[0] == 'ff':
                    fwd_filter(e[1], e[2], plan)
                elif e[0] == 'fd':
                    fwd_data(e[1], e[2], kvs[i], plan)
                elif e[0] == 'dma':
                    plan.put(max(done[0], plan.pos), 0, lambda c=e[1]: (c.start(), [])[1])
                else:
                    place(i, a_fn[e[0]](e[1], e[2], e[3], plan))
            plan.finish()

        def a_work(p):
            h = p % 2
            if p in (4, 5):
                res = [(u + c * MC / D, ('q', c * MC, MC, h * 8 + u)) for u in range(8) for c in range(D // MC)]
                for g in range(h * 4, h * 4 + 4):
                    res += [(2 * (g % 4) + 0.3, ('kv', g)), (2 * (g % 4) + 1.3, ('m', g))]
                return res
            if p >= 6:
                res = []
                for (r0, n), cp in zip(orows, cp_oa):
                    if r0 // D == h:
                        t0 = (r0 % D) / 128
                        res += [(t0 + it * n / D, ('o', r0, n, it)) for it in range(8)]
                        res.append((t0 + 7.5 * n / D, ('dma', cp)))
                return res
            mc = XC if p == 0 else MC
            return [((c * 8 + it) * mc / D, ('kp'[p // 2], h * D + c * mc, mc, it))
                    for c in range(D // mc) for it in range(8)]

        def spread(t0, t1, es):
            return [(t0 + (n + 0.5) * (t1 - t0) / len(es), e) for n, e in enumerate(es)]

        def fwd_work(g):
            return [(kind, g, it) for it in range(4) for kind in ('ff', 'fd')]

        def all_macs(g):
            return sum([mac_items(g, it) for it in range(8)], [])

        grp = lambda g: [cp_s[g], cp_k[g], cp_v[g]]
        order1 = [cp_inv, cp_d, cp_q[0]] + grp(2) + cp_x[3]
        order2 = [cp_q[1], cp_wq] + grp(3)
        order3 = cp_q[2:] + sum([grp(g) for g in range(4, NG)], []) + [cp_wv, cp_wo]

        def wait(cs):
            for c in cs:
                c.wait()

        nw = len(cp_wk)
        work0 = a_work(0) + spread(4, 8, [('fd', 1, it) for it in range(4)])
        macs = all_macs(0)
        cuts = [2 * j / nw for j in range(nw + 1)] + [4, 8]
        stages = [([cp_fwd, cp_msk, cp_s[0]], spread(0, 1, [('ff', 0, it) for it in range(4)]), []),
                  ([cp_s[1]], spread(0, 1, [('ff', 1, it) for it in range(4)]), []),
                  ([cp_sk, cp_k[0], cp_v[0]], spread(0, 1, [('fd', 0, it) for it in range(4)]), [])]
        needs = [cp_x[0] + [cp_wk[0]]] + [[c] for c in cp_wk[1:]] + [cp_x[1], [cp_k[1], cp_v[1]] + cp_x[2]]
        for need, t0, t1 in zip(needs, cuts, cuts[1:]):
            stages.append((need, [e for e in work0 if t0 <= e[0] < t1],
                           [(macs[int(len(macs) * t0 / 8):int(len(macs) * t1 / 8)], t0, t1, False)]))
        queue = [st[0] for st in stages] + [order1 + order2 + order3]
        for cs in queue[:depth]:
            for c in cs:
                c.start()
        kf_v[:, pl.ds(0, HALO), :] = jnp.zeros((2, HALO, 128), F32)
        for j, (need, work, vec) in enumerate(stages):
            wait(need)
            for cs in queue[depth + j:depth + j + 1]:
                for c in cs:
                    c.start()
            if j == 0:
                fu_v[...] = _pack(fwd_v[...])
                zv = jnp.where(msk_v[0:16, :].astype(F32) > -1.0, 0, 1)
                zeros.extend(zv[i, 0] for i in range(16))
            block(work, vec)

        for p in range(1, 8):
            if p == 1:
                wait(order1)
                gu_v[...] = _pack(inv_v[...])
            if p == 2:
                wait(order2)
            if p == 3:
                wait(order3)
            work, vec = a_work(p), []
            if p < 7:
                work += spread(0, 8, fwd_work(p + 1))
                work += spread(0.2, 8.2 - 0.6, [('inv', p - 1, it) for it in range(4)] + [('dma', cp_ob[p - 1])])
                mac_end = 8
            else:
                work += spread(0, 4, [('inv', 6, it) for it in range(4)] + [('dma', cp_ob[6])])
                work += spread(tail[0] + 0.1, tail[1], [('inv', 7, it) for it in range(4)] + [('dma', cp_ob[7])])
                mac_end = tail[0]
            if p in (2, 3):
                vec.append((sum([prep_items(p % 2, it) for it in range(8)], []), 0.2, 7.8, True))
            vec.append((all_macs(p), 0, mac_end, False))
            for j in range(nsub):
                t0, t1 = 8 * j / nsub, 8 * (j + 1) / nsub if j + 1 < nsub else 9
                part = []
                for items, f, l, even in vec:
                    lo, hi = max(t0, f), min(t1, l)
                    if lo < hi:
                        cut = lambda t: round(len(items) * (t - f) / (l - f))
                        part.append((items[cut(lo):cut(hi)], lo, hi, even))
                block([e for e in work if t0 <= e[0] < t1], part)
        wait(cp_ob + cp_oa)

    @jax.jit
    def run(A_x, A_wqkv, A_wo, B_q, B_k, B_v, B_shift_k, B_ssm_k, B_ssm_D):
        fwd, inv, msk = _consts()
        any_spec = pl.BlockSpec(memory_space=pl.ANY)
        vm = pltpu.VMEM
        out = pl.pallas_call(
            kernel,
            out_shape=jax.ShapeDtypeStruct((S, 2 * D), BF16),
            in_specs=[any_spec] * 12,
            out_specs=any_spec,
            scratch_shapes=[
                vm((NG, S, 128), BF16), vm((D, 3 * D), BF16), vm((D, D), BF16),
                vm((NG, S, 128), BF16), vm((NG, S, 128), BF16), vm((NG, S, 128), BF16),
                vm((KS, D), BF16), vm((NG, 128, S), BF16), vm((D,), BF16),
                vm((2 * T, T), BF16), vm((T, T), BF16), vm((128, 128), BF16),
                vm((T, T), U32), vm((T // 2, T), U32), vm((2, HALO + S // 2, 128), F32),
                vm((D // 2, S), U32), vm((D // 2, D), U32), vm((NG, 8, 128), F32), vm((D // 2, D), U32), vm((D, 128), F32),
                vm((S // 2, D), U32), vm((D, D), BF16), vm((S, D), BF16), vm((NG, S, 128), BF16),
                pltpu.SemaphoreType.DMA((96,)), pltpu.SemaphoreType.REGULAR,
            ] + [vm((S // 2, 128), U32)] * 3 + [vm((NB, 2 * T, 128), F32)] * 4 + [vm((NB, T, 128), U32)] * 2,
            compiler_params=pltpu.CompilerParams(vmem_limit_bytes=100 * 1024 * 1024, flags=flags),
        )(A_x.reshape(S, D), A_wqkv, A_wo, B_q.reshape(S, D), B_k.reshape(S, D), B_v.reshape(S, D),
          B_shift_k.T, B_ssm_k, B_ssm_D,
          jnp.asarray(fwd, BF16), jnp.asarray(inv, BF16), jnp.asarray(msk, BF16))
        return out.reshape(1, S, 2 * D)

    return run


pallas_concat_heads__linear_attn_block__ssm_conv_h3__prompt_kernel = make()
```

```python
import functools
import numpy as np
import jax
import jax.numpy as jnp
from jax import lax
from jax.experimental import pallas as pl
from jax.experimental.pallas import tpu as pltpu

S = 2048
D = 1024
DH = 32
T = 128
NB = S // T
NG = D // 128
KS = 4
HALO = 8
F32 = jnp.float32
BF16 = jnp.bfloat16
U32 = jnp.uint32


def _consts():
    ang = 2.0 * np.pi * np.outer(np.arange(T) + 0.25, np.arange(T)) / T
    fwd = np.stack([np.cos(ang), np.sin(ang)], axis=1)
    fwd = fwd.reshape(2, T // 16, 8, 2, T).transpose(1, 0, 3, 2, 4).reshape(2 * T, T)
    inv = np.stack([np.cos(ang), np.sin(ang)], axis=1)[:T // 2].reshape(T, T).T / T
    inv = np.concatenate([inv[0::2], inv[1::2]], axis=0)
    lane = np.arange(128) // DH
    head_mask = (lane[:, None] == lane[None, :]).astype(np.float32)
    return fwd.astype(np.float32), inv.astype(np.float32), head_mask


def _phi(t):
    return jnp.where(t > 0, t + 1.0, jnp.exp(t)) + 1e-6


def _recip(d):
    r = pl.reciprocal(d, approx=True)
    return r * (2.0 - d * r)


def _aligned(i, n):
    return i if isinstance(i, int) else pl.multiple_of(i, n)


def _pack(x):
    return pltpu.bitcast(x, U32)


def _unpack(x):
    return pltpu.bitcast(x, BF16)


def _split(w):
    return [pltpu.unpack_elementwise(w, index=i, packed_dtype=BF16, unpacked_dtype=F32) for i in range(2)]


def _merge(even, odd):
    return pltpu.pack_elementwise([even, odd], packed_dtype=BF16)


def _dot(a, b):
    return jnp.dot(a, b, preferred_element_type=F32)


class _No:
    def start(self): pass
    def wait(self): pass


def make(unroll=1, dma=True, periods=range(8), flags=None, rep=None, tie=True, MC=1024, lag=3, barrier='sem', nsub=1, scopes=False, gate_every=0, gate_shift=0, tie_st=False, WT=256, off=(0.1, 0.2, 0.3), x3_cut=8, defer=0, wide='fd', pad=(0, 0), skip=0, chains=1, split=False, tb=(4, 8, 16, 24, 32, 40, 48, 56, 61, 63), c0=3.5, c1=5.5, ahead=8, tail=(5, 7), orows=((0, 1024, (0, 8)), (1024, 1024, (0, 4, 6, 7, 8)))):
    def kernel(x_h, wqkv_h, wo_h, q_h, k_h, v_h, sk_h, ssm_h, d_h, fwd_h, inv_h, msk_h, out_h,
               x_v, w_v, wo_v, q_v, k_v, v_v, sk_v, ssm_v, d_v, fwd_v, inv_v, msk_v,
               fu_v, gu_v, kf_v, pkt_v, pacc_v, p_v, z_v, wqt_v, zc_v, pqn_v, m_v, oa_v, ob_v, sems, bar, *rest):
        kv_v, xs_v, ks_v, zs_v = rest[0:3], rest[3:5], rest[5:7], rest[7:9]
        sem_ids = {}

        def copy(name, src, dst):
            if not dma:
                return _No()
            if name not in sem_ids:
                sem_ids[name] = len(sem_ids)
            return pltpu.make_async_copy(src, dst, sems.at[sem_ids[name]])

        d_row = lambda g: d_v[...].astype(F32)[g * 128:(g + 1) * 128].reshape(1, 128)
        cols = lambda g: pl.ds(g * 128, 128)
        xw_v, ku_v, vu_v, qu_v, obu_v = [r.bitcast(U32) for r in (x_v, k_v, v_v, q_v, ob_v)]
        XC = 256
        cp_x = [[copy(("x", r0, g), x_h.at[pl.ds(r0, n), cols(g)], x_v.at[g, pl.ds(r0, n)]) for g in range(NG)]
                for r0, n in ((0, XC), (XC, XC), (2 * XC, 2 * XC), (4 * XC, S - 4 * XC))]
        wcols = [(D + j * WT, WT) for j in range(D // WT)] + [(0, D), (2 * D, D)]
        cp_w = [copy(("w", j), wqkv_h.at[:, pl.ds(c0, n)], w_v.at[:, pl.ds(c0, n)]) for j, (c0, n) in enumerate(wcols)]
        cp_wk, cp_wq, cp_wv = cp_w[:-2], cp_w[-2], cp_w[-1]
        cp_wo = copy("wo", wo_h, wo_v)
        cp_q = [copy(("q", g), q_h.at[:, cols(g)], q_v.at[g]) for g in range(NG)]
        cp_k = [copy(("k", g), k_h.at[:, cols(g)], k_v.at[g]) for g in range(NG)]
        cp_v = [copy(("v", g), v_h.at[:, cols(g)], v_v.at[g]) for g in range(NG)]
        cp_s = [copy(("s", g), ssm_h.at[cols(g)], ssm_v.at[g]) for g in range(NG)]
        cp_sk, cp_d, cp_fwd = copy("sk", sk_h, sk_v), copy("d", d_h, d_v), copy("fwd", fwd_h, fwd_v)
        cp_inv, cp_msk = copy("inv", inv_h, inv_v), copy("msk", msk_h, msk_v)
        cp_ob = [copy(("ob", g), ob_v.at[g], out_h.at[:, pl.ds(D + g * 128, 128)]) for g in range(NG)]
        cp_oa = [[copy(("oa", r0, c0), oa_v.at[pl.ds(r0, n), pl.ds(c0 * 128, (c1 - c0) * 128)],
                       out_h.at[pl.ds(r0, n), pl.ds(c0 * 128, (c1 - c0) * 128)]) for c0, c1 in zip(cc, cc[1:])]
                 for r0, n, cc in orows]

        class Plan:
            def __init__(self, nslots):
                self.keep = msk_v[0:8, :].astype(F32) > -1.0
                self.load = [0.0] * nslots
                self.items = [[] for _ in range(nslots)]
                self.pos = 0
                self.prev, self.span, self.gated = None, (0, 1), {}

            def started(self, nslots):
                self.span = (self.pos, nslots)

            def put(self, slot, cost, fn):
                slot = min(slot, len(self.load) - 1)
                self.load[slot] += cost
                self.items[slot].append(fn)

            def spread(self, lo, hi, items):
                for n, (cost, fn) in enumerate(items):
                    self.put(lo + (n * (hi - lo)) // len(items), cost, fn)

            def fill(self, lo, hi, items):
                total = sum(c for c, _ in items)
                level = (total + sum(self.load[lo:hi])) / (hi - lo)
                while sum(max(level - l, 0.0) for l in self.load[lo:hi]) > total:
                    level -= 0.25
                slot, room = lo, 0.0
                room = max(level - self.load[lo], 0.0)
                for cost, fn in items:
                    while room < cost / 2 and slot < hi - 1:
                        slot += 1
                        room += max(level - self.load[slot], 0.0)
                    room -= cost
                    self.put(slot, cost, fn)

            def slab(self, val, step):
                toks = []
                for _ in range(step):
                    for fn in self.items[self.pos]:
                        toks += fn()
                    self.pos += 1
                if not toks or not tie:
                    return val
                for tk in toks:
                    val = jnp.where(self.keep, val, tk if tk.dtype == U32 else pltpu.bitcast(tk, U32))
                return val

            def lhs(self, val, step=1):
                m, k = val.shape
                parts = []
                for c in range(0, k, 512):
                    parts.append(jnp.concatenate(
                        [self.slab(val[r:r + 8, c:c + 128], step) for r in range(0, m, 8)], axis=0))
                    if min(c + 512, k) > c + 128:
                        parts.append(val[:, c + 128:min(c + 512, k)])
                return _unpack(parts[0] if len(parts) == 1 else jnp.concatenate(parts, axis=1))

            def finish(self):
                assert self.pos == len(self.load) - 1, (self.pos, len(self.load))
                for fn in self.items[self.pos]:
                    fn()

        zeros, cur = [], [None]

        def rows_at(r0, n, salt):
            return pl.ds(pl.multiple_of(r0 + zeros[salt % len(zeros)], 8), n)

        def pre_items(g, it, kvs, plan):
            w = sk_v[:, cols(g)].astype(F32)
            w0, w1, w2, w3 = [jnp.broadcast_to(w[tau:tau + 1], (8, 128)) for tau in range(KS)]

            def item(n):
                def fn():
                    r0 = it * T + n * 8
                    for r in range(0 if r0 == 0 else r0 + ahead, min(r0 + ahead + 8, S // 2), 8):
                        for j, kk in enumerate(_split(ku_v[g, pl.ds(r, 8), :])):
                            kf_v[j, pl.ds(HALO + r, 8), :] = kk
                    ve, vo = _split(vu_v[g, pl.ds(r0, 8), :])
                    ke = kf_v[0, pl.ds(HALO + r0, 8), :]
                    ko = kf_v[1, pl.ds(HALO + r0, 8), :]
                    ke1 = kf_v[0, pl.ds(HALO + r0 - 1, 8), :]
                    ko1 = kf_v[1, pl.ds(HALO + r0 - 1, 8), :]
                    ko2 = kf_v[1, pl.ds(HALO + r0 - 2, 8), :]
                    se = (ke * w0 + ko1 * w1) + (ke1 * w2 + ko2 * w3)
                    so = (ko * w0 + ke * w1) + (ko1 * w2 + ke1 * w3)
                    kv = _merge(se * ve, so * vo)
                    kv_v[g % 3][pl.ds(r0, 8), :] = kv
                    kvs.append(kv)
                    return [kv]
                return (22, fn)
            return [item(n) for n in range(2 * T // 16)]

        def fwd_filter(g, it, plan):
            if 'f' in wide:
                flt = jnp.concatenate([ssm_v[g, :, pl.ds((it * 4 + b) * T, T)] for b in range(4)], axis=0)
                res = lax.dot_general(plan.lhs(fu_v[rows_at(0, T, it), :]), flt,
                                      (((1,), (1,)), ((), ())), preferred_element_type=F32)
                for b in range(4):
                    ks_v[g % 2][it * 4 + b] = res[:, b * 128:(b + 1) * 128]
                return
            for b in range(it * 4, it * 4 + 4):
                f = fu_v[rows_at(0, T, b), :]
                ks_v[g % 2][b] = lax.dot_general(
                    plan.lhs(f) if b % 4 == 0 else _unpack(f), ssm_v[g, :, pl.ds(b * T, T)],
                    (((1,), (1,)), ((), ())), preferred_element_type=F32)

        def fwd_data(g, it, kvs, plan):
            if 'd' in wide:
                dat = jnp.concatenate([jnp.concatenate(kvs[b * 8:(b + 1) * 8], axis=0) for b in range(4)], axis=1)
                res = _dot(plan.lhs(fu_v[rows_at(0, T, it + 4), :]), _unpack(dat))
                for b in range(4):
                    xs_v[g % 2][it * 4 + b] = res[:, b * 128:(b + 1) * 128]
                return
            for b in range(4):
                f = fu_v[rows_at(0, T, it * 4 + b + 8), :]
                xs_v[g % 2][it * 4 + b] = _dot(plan.lhs(f) if b == 0 else _unpack(f),
                                               _unpack(jnp.concatenate(kvs[b * 8:(b + 1) * 8], axis=0)))

        def mac_items(g, it):
            s = g % 2
            items, low = [], []
            half = NB // 2 if split else NB
            steps = [(i, 0, min(i + 1, half)) for i in range(NB)] + [(i, half, i + 1) for i in range(half, NB)]
            for pp in range(2):
                st = dict(res=[[], [], []])
                for part in range(3):
                    for i, j0, j1 in steps:
                        def fn(pp=pp, part=part, i=i, j0=j0, j1=j1, st=st):
                            r0 = (it * 2 + pp) * 16

                            def operand(ref, j):
                                key = (id(ref), part, j, j0)
                                if key not in st:
                                    at = lambda r: rows_at(r, 8, it) if j0 and ref is ks_v[s] else pl.ds(r, 8)
                                    vals = [ref[j, at(r0 + 8 * c), :] for c in ((0,), (1,), (0, 1))[part]]
                                    st[key] = vals[0] if part < 2 else vals[0] + vals[1]
                                return st[key]

                            acc = st.pop(('acc', i)) if j0 else None
                            sums = [acc] if j0 else []
                            for j in range(j0, j1):
                                term = operand(ks_v[s], i - j) * operand(xs_v[s], j)
                                if len(sums) < chains:
                                    sums.append(term)
                                else:
                                    sums[j % chains] = sums[j % chains] + term
                            while len(sums) > 1:
                                sums = [sums[n] + sums[n + 1] if n + 1 < len(sums) else sums[n]
                                        for n in range(0, len(sums), 2)]
                            acc = sums[0]
                            if j1 <= i:
                                st['acc', i] = acc
                                return [acc]
                            if part < 2:
                                st['res'][part].append(acc)
                                return [acc] if i >= skip else []
                            p1, p2 = st['res'][0][i], st['res'][1][i]
                            yr, yi = p1 - p2, acc - (p1 + p2)
                            zr = yr if i == 0 else yr + st['yi']
                            zi = yi if i == 0 else yi - st['yr']
                            st['yr'], st['yi'] = yr, yi
                            if pp == 0:
                                low.append((zr, zi))
                                return [zr if i % 2 else zi]
                            ar, ai = low[i]
                            ze, zo = _merge(ar + zr, ai + zi), _merge(ar - zr, ai - zi)
                            zs_v[s][i, pl.ds(it * 8, 8), :] = ze
                            zs_v[s][i, pl.ds(T // 2 + it * 8, 8), :] = zo
                            return [zo if i % 2 else ze]
                        items.append((2 * (j1 - j0) + (7 + 6 * pp if part == 2 and j1 > i else 0), fn))
            return items

        def inv_dots(g, it, plan):
            ys = []
            if 'i' in wide:
                for h in range(2):
                    zz = jnp.concatenate([zs_v[g % 2][it * 4 + b, pl.ds(h * T // 2, T // 2), :] for b in range(4)], axis=1)
                    ys.append(_dot(plan.lhs(gu_v[rows_at(h * T // 4, T // 4, it), :]), _unpack(zz)))
                return [ys[n % 2][:, (n // 2) * 128:(n // 2 + 1) * 128] for n in range(8)]
            for n in range(8):
                half = (n % 2) * (T // 2)
                gm = gu_v[rows_at(half // 2, T // 4, it * 8 + n), :]
                ys.append(_dot(plan.lhs(gm) if n % 4 == 0 else _unpack(gm),
                               _unpack(zs_v[g % 2][it * 4 + n // 2, pl.ds(half, T // 2), :])))
            return ys

        def inv_items(g, it, ys):
            dd = jnp.broadcast_to(d_row(g), (8, 128))

            def item(n):
                def fn():
                    rows = pl.ds(it * 2 * T + n * 8, 8)
                    ye, yo = [ys[(n // 8) * 2 + j][(n % 8) * 8:(n % 8 + 1) * 8] for j in range(2)]
                    kve, kvo = _split(kv_v[g % 3][rows, :])
                    qe, qo = _split(qu_v[g, rows, :])
                    ob = _merge(qe * (ye + kve * dd), qo * (yo + kvo * dd))
                    obu_v[g, rows, :] = ob
                    return [ob]
                return (12, fn)
            return [item(n) for n in range(4 * T // 16)]

        def lanes(it, base=0):
            return pl.ds(base + it * 128, 128)

        def a_k(r0, mc, it, plan):
            st = {}
            rows = rows_at(r0 // 2, mc // 2, it)
            xu = jnp.concatenate([xw_v[g, rows, :] for g in range(NG)], axis=1)
            res = _dot(plan.lhs(xu), w_v[:, lanes(it, D)])
            pks = []
            plan.prev = res

            def item(n):
                def fn():
                    pk = _phi(res[n * 16:(n + 1) * 16])
                    part = pk[0:8] + pk[8:16]
                    st['z'] = part if 'z' not in st else st['z'] + part
                    pks.append(pk)
                    if n % 8 < 7:
                        return [part]
                    pkt = jnp.concatenate(pks[-8:], axis=0).astype(BF16).T
                    pkt_v[pl.ds(it * 64, 64), pl.ds(r0 + (n // 8) * 128, 128)] = _pack(pkt)
                    if n == mc // 16 - 1:
                        z_v[it] = st['z'] if r0 == 0 else z_v[it] + st['z']
                    return [part]
                return (20, fn)
            return [item(n) for n in range(mc // 16)]

        def a_p(s0, mc, it, plan):
            res = _dot(plan.lhs(pkt_v[rows_at(0, D // 2, it), pl.ds(s0, S // 2)]),
                       _unpack(xw_v[it, pl.ds(s0 // 2, S // 4), :]))

            def item(n):
                def fn():
                    part = res[n * 16:(n + 1) * 16]
                    if s0 == 0:
                        pacc_v[it, pl.ds(n * 16, 16), :] = part
                        return []
                    part = part + pacc_v[it, pl.ds(n * 16, 16), :]
                    pb = _merge(part[0:8], part[8:16])
                    p_v[pl.ds(n * 8, 8), lanes(it)] = pb
                    return [pb] if tie_st else []
                return (2, fn)
            return [item(n) for n in range(mc // 16)]

        def prep_items(h, it):
            def wq(n):
                def fn():
                    r0 = h * (D // 2) + n * 128
                    blk = _pack(w_v[pl.ds(r0, 128), lanes(it)].T)
                    wqt_v[pl.ds(it * 64, 64), pl.ds(r0, 128)] = blk
                    return [blk[56:64]]
                return (4, fn)

            def zc():
                z = jnp.sum(z_v[it], axis=0, keepdims=True)
                col = jnp.broadcast_to(z, (128, 128)).T
                zc_v[lanes(it), :] = col
                return [col[120:128]]
            return [wq(n) for n in range(4)] + ([(8, zc)] if h == 1 else [])

        def a_q(f0, mc, it, plan):
            rows = pl.ds(it * 64, 64)
            xr = rows_at(it * 64, 64, f0 // mc)
            xu = jnp.concatenate([xw_v[g, xr, :] for g in range(NG)], axis=1)
            res = lax.dot_general(plan.lhs(wqt_v[rows_at(f0 // 2, mc // 2, it), :]), _unpack(xu),
                                  (((1,), (1,)), ((), ())), preferred_element_type=F32)
            outs = []
            plan.prev = res

            def item(n):
                def fn():
                    pq = _phi(res[n * DH:(n + 1) * DH])
                    pz = pq * zc_v[pl.ds(f0 + n * DH, DH), :]
                    den = (pz[0:8] + pz[8:16]) + (pz[16:24] + pz[24:32])
                    for sh in (4, 2, 1):
                        den = den + pltpu.roll(den, sh, 0)
                    inv = _recip(den + 1e-6)
                    pqn = pq * jnp.concatenate([inv] * 4, axis=0)
                    outs.extend([_merge(pqn[0:8], pqn[8:16]), _merge(pqn[16:24], pqn[24:32])])
                    if n % 4 == 3:
                        pqn_v[rows, pl.ds(f0 + (n // 4) * 128, 128)] = _pack(_unpack(jnp.concatenate(outs[-8:], axis=0)).T)
                    return outs[-2:]
                return (56, fn)
            return [item(n) for n in range(mc // DH)]

        def a_o(r0, mc, it, plan):
            res = _dot(plan.lhs(pqn_v[rows_at(r0 // 2, mc // 2, it), :]), m_v[:, lanes(it)])
            plan.prev = res

            def item(n):
                def fn():
                    ob = res[n * 16:(n + 1) * 16].astype(BF16)
                    oa_v[pl.ds(r0 + n * 16, 16), lanes(it)] = ob
                    return [ob[8:16].astype(F32)] if tie_st else []
                return (2, fn)
            return [item(n) for n in range(mc // 16)]

        a_fn = dict(k=a_k, p=a_p, q=a_q, o=a_o)
        a_cost = dict(k=20 / 16, p=2 / 16, q=28 / 16, o=2 / 16)

        nblk, kvs, carry = [0], {}, []

        def block(work, vec, final):
            nblk[0] += 1
            if barrier == 'sem':
                pl.semaphore_signal(bar, 1)
                pl.semaphore_wait(bar, 1)
            elif barrier == 'delay':
                pl.delay(1)
            if not scopes:
                return block_(work, vec, final)
            with jax.named_scope("blk%02d" % nblk[0]):
                block_(work, vec, final)

        def block_(work, vec, final):
            work = sorted(work, key=lambda e: e[0])
            seq = [e for _, e in work]
            start, n = [], 0
            for e in seq:
                start.append(n)
                n += e[2] // 8 if e[0] in a_fn else dict(kv=16, m=16, inv=8, ff=16, fd=16, dma=0)[e[0]]
            start.append(n)
            slot_at = lambda t: start[sum(1 for tt, _ in work if tt < t)]
            plan = cur[0] = Plan(n + 1)
            if carry:
                plan.spread(0, start[1], list(carry))
                del carry[:]
            late, prev = {}, 0
            for i, e in enumerate(seq):
                lo = min(start[i + 1] + lag, n)
                if e[0] == 'inv':
                    late[i] = (lo, min(lo + 48, n + 1), 12 * 32)
                elif e[0] in a_fn:
                    late[i] = (lo, min(lo + e[2] // 8, n + 1), a_cost[e[0]] * e[2])
                elif e[0] == 'fd':
                    kvs[i] = []
                    lo = max(prev, start[i] - 160)
                    plan.spread(lo, max(start[i] - 8, lo + 1),
                                pre_items(e[1], 2 * e[2], kvs[i], plan) + pre_items(e[1], 2 * e[2] + 1, kvs[i], plan))
                    prev = start[i]
            for lo, hi, cost in late.values():
                for sl in range(lo, hi):
                    plan.load[sl] += cost / (hi - lo)
            for edge in start[1:-1]:
                for sl in range(max(edge - pad[0], 0), min(edge + pad[1], n)):
                    plan.load[sl] += 30
            for items, first, last, even in vec:
                (plan.spread if even else plan.fill)(slot_at(first), max(slot_at(last), slot_at(first) + 1), items)
            done = [0]

            def place(i, items):
                lo, hi, cost = late[i]
                for sl in range(lo, hi):
                    plan.load[sl] -= cost / (hi - lo)
                if lo >= n - defer and not final:
                    carry.extend(items)
                else:
                    plan.spread(lo, hi, items)
                    done[0] = max(done[0], hi - 1)

            for i, e in enumerate(seq):
                if e[0] == 'kv':
                    kvh = _dot(plan.lhs(p_v[pl.ds(e[1] * 64, 64), :]), w_v[:, lanes(e[1], 2 * D)])
                    kvs['head'] = _pack(jnp.where(msk_v[...] > 0, kvh, 0.0).astype(BF16))
                elif e[0] == 'm':
                    for c in range(2):
                        half = pl.ds(c * (D // 2), D // 2)
                        m_v[lanes(e[1]), half] = _dot(plan.lhs(kvs['head']), wo_v[lanes(e[1]), half]).astype(BF16)
                elif e[0] == 'inv':
                    place(i, inv_items(e[1], e[2], inv_dots(e[1], e[2], plan)))
                elif e[0] == 'ff':
                    fwd_filter(e[1], e[2], plan)
                elif e[0] == 'fd':
                    fwd_data(e[1], e[2], kvs[i], plan)
                elif e[0] == 'dma':
                    fn = lambda c=e[1]: (c.start(), [])[1]
                    if carry:
                        carry.append((0, fn))
                    else:
                        plan.put(max(done[0], plan.pos), 0, fn)
                else:
                    place(i, a_fn[e[0]](e[1], e[2], e[3], plan))
            plan.finish()

        def a_work(p):
            h = p % 2
            if p in (4, 5):
                res = [(u + c * MC / D, ('q', c * MC, MC, h * 8 + u)) for u in range(8) for c in range(D // MC)]
                for g in range(h * 4, h * 4 + 4):
                    res += [(2 * (g % 4) + 0.3, ('kv', g)), (2 * (g % 4) + 1.3, ('m', g))]
                return res
            if p >= 6:
                res = []
                for (r0, n, cc), cps in zip(orows, cp_oa):
                    if r0 // D == h:
                        t0 = (r0 % D) / 128
                        res += [(t0 + it * n / D, ('o', r0, n, it)) for it in range(8)]
                        res += [(t0 + (c1 - 0.5) * n / D, ('dma', cp)) for c1, cp in zip(cc[1:], cps)]
                return res
            chunks = ((0, XC), (XC, XC), (2 * XC, D - 2 * XC)) if p == 0 else ((0, D),)
            return [(r0 / 128 + it * mc / D, ('kp'[p // 2], h * D + r0, mc, it))
                    for r0, mc in chunks for it in range(8)]

        def spread(t0, t1, es):
            return [(t0 + (n + 0.5) * (t1 - t0) / len(es), e) for n, e in enumerate(es)]

        def fwd_work(g):
            return [(kind, g, it) for it in range(4) for kind in ('ff', 'fd')]

        def all_macs(g):
            return sum([mac_items(g, it) for it in range(8)], [])

        grp = lambda g: [cp_s[g], cp_k[g], cp_v[g]]
        ff = lambda g: [('ff', g, it) for it in range(4)]
        fd = lambda g: [('fd', g, it) for it in range(4)]
        inv = lambda g: [('inv', g, it) for it in range(4)] + [('dma', cp_ob[g])]

        work, vec = [], []
        for p in range(8):
            work += [(8 * p + t, e) for t, e in a_work(p)]
        work += spread(c0, c0 + 0.2, ff(0)) + spread(c0 + 0.3, 4, fd(0)) + spread(c1, tb[1], fwd_work(1))
        for g in range(NG):
            t0, t1 = tb[g], tb[g + 1]
            if 1 <= g < NG - 1:
                work += spread(t0 + off[0], t1 + off[0], ff(g + 1)) + spread(t0 + off[1], t1 + off[1], fd(g + 1))
                work += spread(t0 + off[2], t1 + off[2], inv(g - 1)[:4]) + [(t1 - 0.1, inv(g - 1)[4])]
            vec.append((all_macs(g), t0, t1, False))
        work += spread(tb[7], tb[8] - 1, inv(6)) + spread(tb[8] + 0.1, tb[9], inv(7))
        vec.append((sum([prep_items(h, it) for h in range(2) for it in range(8)], []), tb[2] + 0.1, 31.5, True))

        nw = len(cp_wk)
        cuts = [(0, [cp_msk] + cp_x[0] + [cp_wk[0]])] + [(2 * j / nw, [cp_wk[j]]) for j in range(1, nw)]
        cuts += [(2, cp_x[1]), (c0, [cp_fwd, cp_sk] + grp(0)), (4, cp_x[2]), (c1, grp(1)),
                 (x3_cut, cp_x[3]), (tb[1], [cp_inv, cp_d, cp_q[0]] + grp(2)),
                 (tb[2], [cp_q[1], cp_wq] + grp(3) + [cp_q[2]] + grp(4)),
                 (tb[3], [cp_wv, cp_wo, cp_q[3]] + grp(5)), (tb[4], cp_q[4:] + grp(6) + grp(7))]
        cuts += [(t, []) for t in tb[5:8]]
        cuts.sort(key=lambda c: c[0])
        ready = lambda cp: next(t for t, need in cuts if any(c is cp for c in need))
        for t, e in work:
            uses = dict(ff=lambda g, _: [cp_fwd, cp_s[g]], fd=lambda g, _: [cp_sk, cp_k[g], cp_v[g]],
                        inv=lambda g, _: [cp_inv, cp_d, cp_q[g]], kv=lambda g: [cp_wv], m=lambda g: [cp_wo])
            assert all(ready(cp) <= t for cp in uses.get(e[0], lambda *_: [])(*e[1:])), (t, e)
        assert ready(cp_wq) <= tb[2] and ready(cp_x[3][0]) <= 8
        for _, need in cuts:
            for c in need:
                c.start()
        kf_v[:, pl.ds(0, HALO), :] = jnp.zeros((2, HALO, 128), F32)
        for (t0, need), t1 in zip(cuts, [t for t, _ in cuts[1:]] + [65]):
            for c in need:
                c.wait()
            if t0 == 0:
                zv = jnp.where(msk_v[0:16, :].astype(F32) > -1.0, 0, 1)
                zeros.extend(zv[i, 0] for i in range(16))
            if t0 == c0:
                fu_v[...] = _pack(fwd_v[...])
            if any(c is cp_inv for c in need):
                gu_v[...] = _pack(inv_v[...])
            part = []
            for items, f, l, even in vec:
                lo, hi = max(t0, f), min(t1, l)
                if lo < hi:
                    cut = lambda t: round(len(items) * (t - f) / (l - f))
                    part.append((items[cut(lo):cut(hi)], lo, hi, even))
            if t1 > t0:
                block([e for e in work if t0 <= e[0] < t1], part, t1 == 65)
        for c in cp_ob + sum(cp_oa, []):
            c.wait()

    @jax.jit
    def run(A_x, A_wqkv, A_wo, B_q, B_k, B_v, B_shift_k, B_ssm_k, B_ssm_D):
        fwd, inv, msk = _consts()
        any_spec = pl.BlockSpec(memory_space=pl.ANY)
        vm = pltpu.VMEM
        out = pl.pallas_call(
            kernel,
            out_shape=jax.ShapeDtypeStruct((S, 2 * D), BF16),
            in_specs=[any_spec] * 12,
            out_specs=any_spec,
            scratch_shapes=[
                vm((NG, S, 128), BF16), vm((D, 3 * D), BF16), vm((D, D), BF16),
                vm((NG, S, 128), BF16), vm((NG, S, 128), BF16), vm((NG, S, 128), BF16),
                vm((KS, D), BF16), vm((NG, 128, S), BF16), vm((D,), BF16),
                vm((2 * T, T), BF16), vm((T, T), BF16), vm((128, 128), BF16),
                vm((T, T), U32), vm((T // 2, T), U32), vm((2, HALO + S // 2, 128), F32),
                vm((D // 2, S), U32), vm((NG, D, 128), F32), vm((D // 2, D), U32), vm((NG, 8, 128), F32), vm((D // 2, D), U32), vm((D, 128), F32),
                vm((S // 2, D), U32), vm((D, D), BF16), vm((S, D), BF16), vm((NG, S, 128), BF16),
                pltpu.SemaphoreType.DMA((96,)), pltpu.SemaphoreType.REGULAR,
            ] + [vm((S // 2, 128), U32)] * 3 + [vm((NB, 2 * T, 128), F32)] * 4 + [vm((NB, T, 128), U32)] * 2,
            compiler_params=pltpu.CompilerParams(vmem_limit_bytes=100 * 1024 * 1024, flags=flags),
        )(A_x.reshape(S, D), A_wqkv, A_wo, B_q.reshape(S, D), B_k.reshape(S, D), B_v.reshape(S, D),
          B_shift_k.T, B_ssm_k, B_ssm_D,
          jnp.asarray(fwd, BF16), jnp.asarray(inv, BF16), jnp.asarray(msk, BF16))
        return out.reshape(1, S, 2 * D)

    return run


pallas_concat_heads__linear_attn_block__ssm_conv_h3__prompt_kernel = make()
```

```python
import functools
import numpy as np
import jax
import jax.numpy as jnp
from jax import lax
from jax.experimental import pallas as pl
from jax.experimental.pallas import tpu as pltpu

S = 2048
D = 1024
DH = 32
T = 128
NB = S // T
NG = D // 128
KS = 4
HALO = 8
F32 = jnp.float32
BF16 = jnp.bfloat16
U32 = jnp.uint32


def _consts():
    ang = 2.0 * np.pi * np.outer(np.arange(T) + 0.25, np.arange(T)) / T
    fwd = np.stack([np.cos(ang), np.sin(ang)], axis=1)
    fwd = fwd.reshape(2, T // 16, 8, 2, T).transpose(1, 0, 3, 2, 4).reshape(2 * T, T)
    inv = np.stack([np.cos(ang), np.sin(ang)], axis=1)[:T // 2].reshape(T, T).T / T
    inv = np.concatenate([inv[0::2], inv[1::2]], axis=0)
    lane = np.arange(128) // DH
    head_mask = (lane[:, None] == lane[None, :]).astype(np.float32)
    return fwd.astype(np.float32), inv.astype(np.float32), head_mask


def _phi(t):
    return jnp.where(t > 0, t + 1.0, jnp.exp(t)) + 1e-6


def _recip(d):
    r = pl.reciprocal(d, approx=True)
    return r * (2.0 - d * r)


def _aligned(i, n):
    return i if isinstance(i, int) else pl.multiple_of(i, n)


def _pack(x):
    return pltpu.bitcast(x, U32)


def _unpack(x):
    return pltpu.bitcast(x, BF16)


def _split(w):
    return [pltpu.unpack_elementwise(w, index=i, packed_dtype=BF16, unpacked_dtype=F32) for i in range(2)]


def _merge(even, odd):
    return pltpu.pack_elementwise([even, odd], packed_dtype=BF16)


def _dot(a, b):
    return jnp.dot(a, b, preferred_element_type=F32)


class _No:
    def start(self): pass
    def wait(self): pass


def make(unroll=1, dma=True, periods=range(8), flags=None, rep=None, tie=True, MC=1024, lag=3, barrier='sem', nsub=1, scopes=False, gate_every=0, gate_shift=0, tie_st=False, wcut=(0, 2, 4, 6, 8), off=(0.1, 0.2, 0.3), x3_cut=8, defer=0, wide='fd', pad=(0, 0), skip=0, chains=1, split=False, tb=(4, 11, 19, 26, 33, 40, 48, 56, 61, 63), c0=3.5, c1=5.5, ahead=8, tail=(5, 7), orows=((0, 1024, (0, 8)), (1024, 1024, (0, 4, 6, 7, 8)))):
    def kernel(x_h, wqkv_h, wo_h, q_h, k_h, v_h, sk_h, ssm_h, d_h, fwd_h, inv_h, msk_h, out_h,
               x_v, wk_v, wq_v, wv_v, wo_v, q_v, k_v, v_v, sk_v, ssm_v, d_v, fwd_v, inv_v, msk_v,
               fu_v, gu_v, kf_v, pk0_v, pk1_v, pacc_v, p_v, z_v, wqt_v, zc_v, pq0_v, pq1_v, m_v, oa_v, ob_v, sems, bar, *rest):
        kv_v, xs_v, ks_v, zs_v = rest[0:3], rest[3:5], rest[5:7], rest[7:9]
        sem_ids = {}

        def copy(name, src, dst):
            if not dma:
                return _No()
            if name not in sem_ids:
                sem_ids[name] = len(sem_ids)
            return pltpu.make_async_copy(src, dst, sems.at[sem_ids[name]])

        d_row = lambda g: d_v[...].astype(F32)[g * 128:(g + 1) * 128].reshape(1, 128)
        cols = lambda g: pl.ds(g * 128, 128)
        xw_v, ku_v, vu_v, qu_v, obu_v = [r.bitcast(U32) for r in (x_v, k_v, v_v, q_v, ob_v)]
        XC = 256
        cp_x = [[copy(("x", r0, g), x_h.at[pl.ds(r0, n), cols(g)], x_v.at[g, pl.ds(r0, n)]) for g in range(NG)]
                for r0, n in ((0, XC), (XC, XC), (2 * XC, 2 * XC), (4 * XC, S - 4 * XC))]
        cp_wk = [copy(("wk", g), wqkv_h.at[:, pl.ds(D + g * 128, 128)], wk_v.at[g]) for g in range(NG)]
        cp_wq = copy("wq", wqkv_h.at[:, pl.ds(0, D)], wq_v)
        cp_wv = copy("wv", wqkv_h.at[:, pl.ds(2 * D, D)], wv_v)
        cp_wo = copy("wo", wo_h, wo_v)
        cp_q = [copy(("q", g), q_h.at[:, cols(g)], q_v.at[g]) for g in range(NG)]
        cp_k = [copy(("k", g), k_h.at[:, cols(g)], k_v.at[g]) for g in range(NG)]
        cp_v = [copy(("v", g), v_h.at[:, cols(g)], v_v.at[g]) for g in range(NG)]
        cp_s = [copy(("s", g), ssm_h.at[cols(g)], ssm_v.at[g]) for g in range(NG)]
        cp_sk, cp_d, cp_fwd = copy("sk", sk_h, sk_v), copy("d", d_h, d_v), copy("fwd", fwd_h, fwd_v)
        cp_inv, cp_msk = copy("inv", inv_h, inv_v), copy("msk", msk_h, msk_v)
        cp_ob = [copy(("ob", g), ob_v.at[g], out_h.at[:, pl.ds(D + g * 128, 128)]) for g in range(NG)]
        cp_oa = [[copy(("oa", r0, c0), oa_v.at[pl.ds(r0, n), pl.ds(c0 * 128, (c1 - c0) * 128)],
                       out_h.at[pl.ds(r0, n), pl.ds(c0 * 128, (c1 - c0) * 128)]) for c0, c1 in zip(cc, cc[1:])]
                 for r0, n, cc in orows]

        class Plan:
            def __init__(self, nslots):
                self.keep = msk_v[0:8, :].astype(F32) > -1.0
                self.load = [0.0] * nslots
                self.items = [[] for _ in range(nslots)]
                self.pos = 0
                self.prev, self.span, self.gated = None, (0, 1), {}

            def started(self, nslots):
                self.span = (self.pos, nslots)

            def put(self, slot, cost, fn):
                slot = min(slot, len(self.load) - 1)
                self.load[slot] += cost
                self.items[slot].append(fn)

            def spread(self, lo, hi, items):
                for n, (cost, fn) in enumerate(items):
                    self.put(lo + (n * (hi - lo)) // len(items), cost, fn)

            def fill(self, lo, hi, items):
                total = sum(c for c, _ in items)
                level = (total + sum(self.load[lo:hi])) / (hi - lo)
                while sum(max(level - l, 0.0) for l in self.load[lo:hi]) > total:
                    level -= 0.25
                slot, room = lo, 0.0
                room = max(level - self.load[lo], 0.0)
                for cost, fn in items:
                    while room < cost / 2 and slot < hi - 1:
                        slot += 1
                        room += max(level - self.load[slot], 0.0)
                    room -= cost
                    self.put(slot, cost, fn)

            def slab(self, val, step):
                toks = []
                for _ in range(step):
                    for fn in self.items[self.pos]:
                        toks += fn()
                    self.pos += 1
                if not toks or not tie:
                    return val
                for tk in toks:
                    val = jnp.where(self.keep, val, tk if tk.dtype == U32 else pltpu.bitcast(tk, U32))
                return val

            def lhs(self, val, step=1):
                m, k = val.shape
                parts = []
                for c in range(0, k, 512):
                    parts.append(jnp.concatenate(
                        [self.slab(val[r:r + 8, c:c + 128], step) for r in range(0, m, 8)], axis=0))
                    if min(c + 512, k) > c + 128:
                        parts.append(val[:, c + 128:min(c + 512, k)])
                return _unpack(parts[0] if len(parts) == 1 else jnp.concatenate(parts, axis=1))

            def finish(self):
                assert self.pos == len(self.load) - 1, (self.pos, len(self.load))
                for fn in self.items[self.pos]:
                    fn()

        zeros, cur = [], [None]

        def rows_at(r0, n, salt):
            return pl.ds(pl.multiple_of(r0 + zeros[salt % len(zeros)], 8), n)

        def pre_items(g, it, kvs, plan):
            w = sk_v[:, cols(g)].astype(F32)
            w0, w1, w2, w3 = [jnp.broadcast_to(w[tau:tau + 1], (8, 128)) for tau in range(KS)]

            def item(n):
                def fn():
                    r0 = it * T + n * 8
                    for r in range(0 if r0 == 0 else r0 + ahead, min(r0 + ahead + 8, S // 2), 8):
                        for j, kk in enumerate(_split(ku_v[g, pl.ds(r, 8), :])):
                            kf_v[j, pl.ds(HALO + r, 8), :] = kk
                    ve, vo = _split(vu_v[g, pl.ds(r0, 8), :])
                    ke = kf_v[0, pl.ds(HALO + r0, 8), :]
                    ko = kf_v[1, pl.ds(HALO + r0, 8), :]
                    ke1 = kf_v[0, pl.ds(HALO + r0 - 1, 8), :]
                    ko1 = kf_v[1, pl.ds(HALO + r0 - 1, 8), :]
                    ko2 = kf_v[1, pl.ds(HALO + r0 - 2, 8), :]
                    se = (ke * w0 + ko1 * w1) + (ke1 * w2 + ko2 * w3)
                    so = (ko * w0 + ke * w1) + (ko1 * w2 + ke1 * w3)
                    kv = _merge(se * ve, so * vo)
                    kv_v[g % 3][pl.ds(r0, 8), :] = kv
                    kvs.append(kv)
                    return [kv]
                return (22, fn)
            return [item(n) for n in range(2 * T // 16)]

        def fwd_filter(g, it, plan):
            if 'f' in wide:
                flt = jnp.concatenate([ssm_v[g, :, pl.ds((it * 4 + b) * T, T)] for b in range(4)], axis=0)
                res = lax.dot_general(plan.lhs(fu_v[rows_at(0, T, it), :]), flt,
                                      (((1,), (1,)), ((), ())), preferred_element_type=F32)
                for b in range(4):
                    ks_v[g % 2][it * 4 + b] = res[:, b * 128:(b + 1) * 128]
                return
            for b in range(it * 4, it * 4 + 4):
                f = fu_v[rows_at(0, T, b), :]
                ks_v[g % 2][b] = lax.dot_general(
                    plan.lhs(f) if b % 4 == 0 else _unpack(f), ssm_v[g, :, pl.ds(b * T, T)],
                    (((1,), (1,)), ((), ())), preferred_element_type=F32)

        def fwd_data(g, it, kvs, plan):
            if 'd' in wide:
                dat = jnp.concatenate([jnp.concatenate(kvs[b * 8:(b + 1) * 8], axis=0) for b in range(4)], axis=1)
                res = _dot(plan.lhs(fu_v[rows_at(0, T, it + 4), :]), _unpack(dat))
                for b in range(4):
                    xs_v[g % 2][it * 4 + b] = res[:, b * 128:(b + 1) * 128]
                return
            for b in range(4):
                f = fu_v[rows_at(0, T, it * 4 + b + 8), :]
                xs_v[g % 2][it * 4 + b] = _dot(plan.lhs(f) if b == 0 else _unpack(f),
                                               _unpack(jnp.concatenate(kvs[b * 8:(b + 1) * 8], axis=0)))

        def mac_items(g, it):
            s = g % 2
            items, low = [], []
            half = NB // 2 if split else NB
            steps = [(i, 0, min(i + 1, half)) for i in range(NB)] + [(i, half, i + 1) for i in range(half, NB)]
            for pp in range(2):
                st = dict(res=[[], [], []])
                for part in range(3):
                    for i, j0, j1 in steps:
                        def fn(pp=pp, part=part, i=i, j0=j0, j1=j1, st=st):
                            r0 = (it * 2 + pp) * 16

                            def operand(ref, j):
                                key = (id(ref), part, j, j0)
                                if key not in st:
                                    at = lambda r: rows_at(r, 8, it) if j0 and ref is ks_v[s] else pl.ds(r, 8)
                                    vals = [ref[j, at(r0 + 8 * c), :] for c in ((0,), (1,), (0, 1))[part]]
                                    st[key] = vals[0] if part < 2 else vals[0] + vals[1]
                                return st[key]

                            acc = st.pop(('acc', i)) if j0 else None
                            sums = [acc] if j0 else []
                            for j in range(j0, j1):
                                term = operand(ks_v[s], i - j) * operand(xs_v[s], j)
                                if len(sums) < chains:
                                    sums.append(term)
                                else:
                                    sums[j % chains] = sums[j % chains] + term
                            while len(sums) > 1:
                                sums = [sums[n] + sums[n + 1] if n + 1 < len(sums) else sums[n]
                                        for n in range(0, len(sums), 2)]
                            acc = sums[0]
                            if j1 <= i:
                                st['acc', i] = acc
                                return [acc]
                            if part < 2:
                                st['res'][part].append(acc)
                                return [acc] if i >= skip else []
                            p1, p2 = st['res'][0][i], st['res'][1][i]
                            yr, yi = p1 - p2, acc - (p1 + p2)
                            zr = yr if i == 0 else yr + st['yi']
                            zi = yi if i == 0 else yi - st['yr']
                            st['yr'], st['yi'] = yr, yi
                            if pp == 0:
                                low.append((zr, zi))
                                return [zr if i % 2 else zi]
                            ar, ai = low[i]
                            ze, zo = _merge(ar + zr, ai + zi), _merge(ar - zr, ai - zi)
                            zs_v[s][i, pl.ds(it * 8, 8), :] = ze
                            zs_v[s][i, pl.ds(T // 2 + it * 8, 8), :] = zo
                            return [zo if i % 2 else ze]
                        items.append((2 * (j1 - j0) + (7 + 6 * pp if part == 2 and j1 > i else 0), fn))
            return items

        def inv_dots(g, it, plan):
            ys = []
            if 'i' in wide:
                for h in range(2):
                    zz = jnp.concatenate([zs_v[g % 2][it * 4 + b, pl.ds(h * T // 2, T // 2), :] for b in range(4)], axis=1)
                    ys.append(_dot(plan.lhs(gu_v[rows_at(h * T // 4, T // 4, it), :]), _unpack(zz)))
                return [ys[n % 2][:, (n // 2) * 128:(n // 2 + 1) * 128] for n in range(8)]
            for n in range(8):
                half = (n % 2) * (T // 2)
                gm = gu_v[rows_at(half // 2, T // 4, it * 8 + n), :]
                ys.append(_dot(plan.lhs(gm) if n % 4 == 0 else _unpack(gm),
                               _unpack(zs_v[g % 2][it * 4 + n // 2, pl.ds(half, T // 2), :])))
            return ys

        def inv_items(g, it, ys):
            dd = jnp.broadcast_to(d_row(g), (8, 128))

            def item(n):
                def fn():
                    rows = pl.ds(it * 2 * T + n * 8, 8)
                    ye, yo = [ys[(n // 8) * 2 + j][(n % 8) * 8:(n % 8 + 1) * 8] for j in range(2)]
                    kve, kvo = _split(kv_v[g % 3][rows, :])
                    qe, qo = _split(qu_v[g, rows, :])
                    ob = _merge(qe * (ye + kve * dd), qo * (yo + kvo * dd))
                    obu_v[g, rows, :] = ob
                    return [ob]
                return (12, fn)
            return [item(n) for n in range(4 * T // 16)]

        def lanes(it, base=0):
            return pl.ds(base + it * 128, 128)

        def a_k(r0, mc, it, plan):
            st = {}
            rows = rows_at(r0 // 2, mc // 2, it)
            xu = jnp.concatenate([xw_v[g, rows, :] for g in range(NG)], axis=1)
            res = _dot(plan.lhs(xu), _unpack(wk_v.bitcast(U32)[it]))
            pks = []
            plan.prev = res

            def item(n):
                def fn():
                    pk = _phi(res[n * 16:(n + 1) * 16])
                    part = pk[0:8] + pk[8:16]
                    st['z'] = part if 'z' not in st else st['z'] + part
                    pks.append(pk)
                    if n % 8 < 7:
                        return [part]
                    pkt = jnp.concatenate(pks[-8:], axis=0).astype(BF16).T
                    (pk0_v, pk1_v)[r0 // D][pl.ds(it * 64, 64), pl.ds(r0 % D + (n // 8) * 128, 128)] = _pack(pkt)
                    if n == mc // 16 - 1:
                        z_v[it] = st['z'] if r0 == 0 else z_v[it] + st['z']
                    return [part]
                return (20, fn)
            return [item(n) for n in range(mc // 16)]

        def a_p(s0, mc, it, plan):
            res = _dot(plan.lhs((pk0_v, pk1_v)[s0 // D][rows_at(0, D // 2, it), :]),
                       _unpack(xw_v[it, pl.ds(s0 // 2, S // 4), :]))

            def item(n):
                def fn():
                    part = res[n * 16:(n + 1) * 16]
                    if s0 == 0:
                        pacc_v[it, pl.ds(n * 16, 16), :] = part
                        return []
                    part = part + pacc_v[it, pl.ds(n * 16, 16), :]
                    pb = _merge(part[0:8], part[8:16])
                    p_v[pl.ds(n * 8, 8), lanes(it)] = pb
                    return [pb] if tie_st else []
                return (2, fn)
            return [item(n) for n in range(mc // 16)]

        def prep_items(h, it):
            def wq(n):
                def fn():
                    r0 = h * (D // 2) + n * 128
                    blk = _pack(wq_v[pl.ds(r0, 128), lanes(it)].T)
                    wqt_v[pl.ds(it * 64, 64), pl.ds(r0, 128)] = blk
                    return [blk[56:64]]
                return (4, fn)

            def zc():
                z = jnp.sum(z_v[it], axis=0, keepdims=True)
                col = jnp.broadcast_to(z, (128, 128)).T
                zc_v[lanes(it), :] = col
                return [col[120:128]]
            return [wq(n) for n in range(4)] if h < 2 else [(8, zc)]

        def a_q(f0, mc, it, plan):
            rows = pl.ds(it % 8 * 64, 64)
            xr = rows_at(it * 64, 64, f0 // mc)
            xu = jnp.concatenate([xw_v[g, xr, :] for g in range(NG)], axis=1)
            res = lax.dot_general(plan.lhs(wqt_v[rows_at(f0 // 2, mc // 2, it), :]), _unpack(xu),
                                  (((1,), (1,)), ((), ())), preferred_element_type=F32)
            outs = []
            plan.prev = res

            def item(n):
                def fn():
                    pq = _phi(res[n * DH:(n + 1) * DH])
                    pz = pq * zc_v[pl.ds(f0 + n * DH, DH), :]
                    den = (pz[0:8] + pz[8:16]) + (pz[16:24] + pz[24:32])
                    for sh in (4, 2, 1):
                        den = den + pltpu.roll(den, sh, 0)
                    inv = _recip(den + 1e-6)
                    pqn = pq * jnp.concatenate([inv] * 4, axis=0)
                    outs.extend([_merge(pqn[0:8], pqn[8:16]), _merge(pqn[16:24], pqn[24:32])])
                    if n % 4 == 3:
                        (pq0_v, pq1_v)[it // 8][rows, pl.ds(f0 + (n // 4) * 128, 128)] = _pack(_unpack(jnp.concatenate(outs[-8:], axis=0)).T)
                    return outs[-2:]
                return (56, fn)
            return [item(n) for n in range(mc // DH)]

        def a_o(r0, mc, it, plan):
            res = _dot(plan.lhs((pq0_v, pq1_v)[r0 // D][rows_at(0, mc // 2, it), :]), m_v[:, lanes(it)])
            plan.prev = res

            def item(n):
                def fn():
                    ob = res[n * 16:(n + 1) * 16].astype(BF16)
                    oa_v[pl.ds(r0 + n * 16, 16), lanes(it)] = ob
                    return [ob[8:16].astype(F32)] if tie_st else []
                return (2, fn)
            return [item(n) for n in range(mc // 16)]

        a_fn = dict(k=a_k, p=a_p, q=a_q, o=a_o)
        a_cost = dict(k=20 / 16, p=2 / 16, q=28 / 16, o=2 / 16)

        nblk, kvs, carry = [0], {}, []

        def block(work, vec, final):
            nblk[0] += 1
            if barrier == 'sem':
                pl.semaphore_signal(bar, 1)
                pl.semaphore_wait(bar, 1)
            elif barrier == 'delay':
                pl.delay(1)
            if not scopes:
                return block_(work, vec, final)
            with jax.named_scope("blk%02d" % nblk[0]):
                block_(work, vec, final)

        def block_(work, vec, final):
            work = sorted(work, key=lambda e: e[0])
            seq = [e for _, e in work]
            start, n = [], 0
            for e in seq:
                start.append(n)
                n += e[2] // 8 if e[0] in a_fn else dict(kv=16, m=16, inv=8, ff=16, fd=16, dma=0)[e[0]]
            start.append(n)
            slot_at = lambda t: start[sum(1 for tt, _ in work if tt < t)]
            plan = cur[0] = Plan(n + 1)
            if carry:
                plan.spread(0, start[1], list(carry))
                del carry[:]
            late, prev = {}, 0
            for i, e in enumerate(seq):
                lo = min(start[i + 1] + lag, n)
                if e[0] == 'inv':
                    late[i] = (lo, min(lo + 48, n + 1), 12 * 32)
                elif e[0] in a_fn:
                    late[i] = (lo, min(lo + e[2] // 8, n + 1), a_cost[e[0]] * e[2])
                elif e[0] == 'fd':
                    kvs[i] = []
                    lo = max(prev, start[i] - 160)
                    plan.spread(lo, max(start[i] - 8, lo + 1),
                                pre_items(e[1], 2 * e[2], kvs[i], plan) + pre_items(e[1], 2 * e[2] + 1, kvs[i], plan))
                    prev = start[i]
            for lo, hi, cost in late.values():
                for sl in range(lo, hi):
                    plan.load[sl] += cost / (hi - lo)
            for edge in start[1:-1]:
                for sl in range(max(edge - pad[0], 0), min(edge + pad[1], n)):
                    plan.load[sl] += 30
            for items, first, last, even in vec:
                (plan.spread if even else plan.fill)(slot_at(first), max(slot_at(last), slot_at(first) + 1), items)
            done = [0]

            def place(i, items):
                lo, hi, cost = late[i]
                for sl in range(lo, hi):
                    plan.load[sl] -= cost / (hi - lo)
                if lo >= n - defer and not final:
                    carry.extend(items)
                else:
                    plan.spread(lo, hi, items)
                    done[0] = max(done[0], hi - 1)

            for i, e in enumerate(seq):
                if e[0] == 'kv':
                    kvh = _dot(plan.lhs(p_v[pl.ds(e[1] * 64, 64), :]), wv_v[:, lanes(e[1])])
                    kvs['head', e[1]] = _pack(jnp.where(msk_v[...] > 0, kvh, 0.0).astype(BF16))
                elif e[0] == 'm':
                    for c in range(2):
                        half = pl.ds(c * (D // 2), D // 2)
                        m_v[lanes(e[1]), half] = _dot(plan.lhs(kvs['head', e[1]]), wo_v[lanes(e[1]), half]).astype(BF16)
                elif e[0] == 'inv':
                    place(i, inv_items(e[1], e[2], inv_dots(e[1], e[2], plan)))
                elif e[0] == 'ff':
                    fwd_filter(e[1], e[2], plan)
                elif e[0] == 'fd':
                    fwd_data(e[1], e[2], kvs[i], plan)
                elif e[0] == 'dma':
                    fn = lambda c=e[1]: (c.start(), [])[1]
                    if carry:
                        carry.append((0, fn))
                    else:
                        plan.put(max(done[0], plan.pos), 0, fn)
                else:
                    place(i, a_fn[e[0]](e[1], e[2], e[3], plan))
            plan.finish()

        def a_work():
            unit = lambda kind, h: [[(kind, h * D, D, it)] for it in range(8)]
            q = [[('q', 0, D, it)] for it in range(16)]
            o = [unit('o', h) for h in range(2)]
            for (_, _, cc), cps, oh in zip(orows, cp_oa, o):
                for c1, cp in zip(cc[1:], cps):
                    oh[c1 - 1].append(('dma', cp))
            res = [(r0 / 128 + it * mc / D, ('k', r0, mc, it))
                   for r0, mc in ((0, XC), (XC, XC), (2 * XC, D - 2 * XC)) for it in range(8)]
            mix = lambda a, b: [u for pair in zip(a, b) for u in pair]
            units = mix(unit('k', 1), unit('p', 0)) + mix(unit('p', 1), q[:8]) + q[8:10]
            units += mix(o[0][:6], q[10:]) + o[0][6:] + o[1]
            res += [(8 + t + j / 2, e) for t, es in enumerate(units) for j, e in enumerate(es)]
            return res + spread(40.1, 41.9, [('kv', 0)] + sum(
                [[('kv', g + 1), ('m', g)] for g in range(NG - 1)], []) + [('m', NG - 1)])

        def spread(t0, t1, es):
            return [(t0 + (n + 0.5) * (t1 - t0) / len(es), e) for n, e in enumerate(es)]

        def fwd_work(g):
            return [(kind, g, it) for it in range(4) for kind in ('ff', 'fd')]

        def all_macs(g):
            return sum([mac_items(g, it) for it in range(8)], [])

        grp = lambda g: [cp_s[g], cp_k[g], cp_v[g]]
        ff = lambda g: [('ff', g, it) for it in range(4)]
        fd = lambda g: [('fd', g, it) for it in range(4)]
        inv = lambda g: [('inv', g, it) for it in range(4)] + [('dma', cp_ob[g])]

        work, vec = a_work(), []
        work += spread(c0, c0 + 0.2, ff(0)) + spread(c0 + 0.3, 4, fd(0)) + spread(c1, tb[1], fwd_work(1))
        for g in range(NG):
            t0, t1 = tb[g], tb[g + 1]
            if 1 <= g < NG - 1:
                work += spread(t0 + off[0], t1 + off[0], ff(g + 1)) + spread(t0 + off[1], t1 + off[1], fd(g + 1))
                work += spread(t0 + off[2], t1 + off[2], inv(g - 1)[:4]) + [(t1 - 0.1, inv(g - 1)[4])]
            vec.append((all_macs(g), t0, t1, False))
        work += spread(tb[7], tb[8] - 1, inv(6)) + spread(tb[8] + 0.1, tb[9], inv(7))
        vec.append((sum([prep_items(h, it) for h in range(2) for it in range(8)], []), tb[2] + 0.1, 23.9, True))
        vec.append((sum([prep_items(2, it) for it in range(8)], []), 24.1, 25.5, True))

        cuts = [(j0 / 4, cp_wk[j0:j1]) for j0, j1 in zip(wcut, wcut[1:])]
        cuts[0] = (0, [cp_msk] + cp_x[0] + cuts[0][1])
        cuts += [(2, cp_x[1]), (c0, [cp_fwd, cp_sk] + grp(0)), (4, cp_x[2]), (c1, grp(1)),
                 (x3_cut, cp_x[3]), (tb[1], [cp_inv, cp_d, cp_q[0]] + grp(2)),
                 (tb[2], [cp_q[1], cp_wq] + grp(3) + [cp_q[2]] + grp(4)),
                 (tb[3], [cp_q[3]] + grp(5)), (tb[4], cp_q[4:] + [cp_wv, cp_wo] + grp(6) + grp(7))]
        cuts += [(t, []) for t in tb[5:8]]
        cuts.sort(key=lambda c: c[0])
        ready = lambda cp: next(t for t, need in cuts if any(c is cp for c in need))
        for t, e in work:
            uses = dict(ff=lambda g, _: [cp_fwd, cp_s[g]], fd=lambda g, _: [cp_sk, cp_k[g], cp_v[g]],
                        inv=lambda g, _: [cp_inv, cp_d, cp_q[g]], kv=lambda g: [cp_wv], m=lambda g: [cp_wo])
            assert all(ready(cp) <= t for cp in uses.get(e[0], lambda *_: [])(*e[1:])), (t, e)
        assert ready(cp_wq) <= tb[2] and ready(cp_x[3][0]) <= 8
        for _, need in cuts:
            for c in need:
                c.start()
        kf_v[:, pl.ds(0, HALO), :] = jnp.zeros((2, HALO, 128), F32)
        for (t0, need), t1 in zip(cuts, [t for t, _ in cuts[1:]] + [65]):
            for c in need:
                c.wait()
            if t0 == 0:
                zv = jnp.where(msk_v[0:16, :].astype(F32) > -1.0, 0, 1)
                zeros.extend(zv[i, 0] for i in range(16))
            if t0 == c0:
                fu_v[...] = _pack(fwd_v[...])
            if any(c is cp_inv for c in need):
                gu_v[...] = _pack(inv_v[...])
            part = []
            for items, f, l, even in vec:
                lo, hi = max(t0, f), min(t1, l)
                if lo < hi:
                    cut = lambda t: round(len(items) * (t - f) / (l - f))
                    part.append((items[cut(lo):cut(hi)], lo, hi, even))
            if t1 > t0:
                block([e for e in work if t0 <= e[0] < t1], part, t1 == 65)
        for c in cp_ob + sum(cp_oa, []):
            c.wait()

    @jax.jit
    def run(A_x, A_wqkv, A_wo, B_q, B_k, B_v, B_shift_k, B_ssm_k, B_ssm_D):
        fwd, inv, msk = _consts()
        any_spec = pl.BlockSpec(memory_space=pl.ANY)
        vm = pltpu.VMEM
        out = pl.pallas_call(
            kernel,
            out_shape=jax.ShapeDtypeStruct((S, 2 * D), BF16),
            in_specs=[any_spec] * 12,
            out_specs=any_spec,
            scratch_shapes=[
                vm((NG, S, 128), BF16), vm((NG, D, 128), BF16), vm((D, D), BF16), vm((D, D), BF16), vm((D, D), BF16),
                vm((NG, S, 128), BF16), vm((NG, S, 128), BF16), vm((NG, S, 128), BF16),
                vm((KS, D), BF16), vm((NG, 128, S), BF16), vm((D,), BF16),
                vm((2 * T, T), BF16), vm((T, T), BF16), vm((128, 128), BF16),
                vm((T, T), U32), vm((T // 2, T), U32), vm((2, HALO + S // 2, 128), F32),
                vm((D // 2, S // 2), U32), vm((D // 2, S // 2), U32), vm((NG, D, 128), F32), vm((D // 2, D), U32), vm((NG, 8, 128), F32), vm((D // 2, D), U32), vm((D, 128), F32),
                vm((S // 4, D), U32), vm((S // 4, D), U32), vm((D, D), BF16), vm((S, D), BF16), vm((NG, S, 128), BF16),
                pltpu.SemaphoreType.DMA((104,)), pltpu.SemaphoreType.REGULAR,
            ] + [vm((S // 2, 128), U32)] * 3 + [vm((NB, 2 * T, 128), F32)] * 4 + [vm((NB, T, 128), U32)] * 2,
            compiler_params=pltpu.CompilerParams(vmem_limit_bytes=100 * 1024 * 1024, flags=flags),
        )(A_x.reshape(S, D), A_wqkv, A_wo, B_q.reshape(S, D), B_k.reshape(S, D), B_v.reshape(S, D),
          B_shift_k.T, B_ssm_k, B_ssm_D,
          jnp.asarray(fwd, BF16), jnp.asarray(inv, BF16), jnp.asarray(msk, BF16))
        return out.reshape(1, S, 2 * D)

    return run


pallas_concat_heads__linear_attn_block__ssm_conv_h3__prompt_kernel = make()
```

```python
import numpy as np
import jax
import jax.numpy as jnp
from jax import lax
from jax.experimental import pallas as pl
from jax.experimental.pallas import tpu as pltpu

S = 2048
D = 1024
DH = 32
T = 128
NB = S // T
NG = D // 128
KS = 4
HALO = 8
LAG = 3
GROUP_TIMES = (4, 11, 18, 26, 34, 42, 49, 56, 61, 63)
OUT_PIECES = ((0, D, (0, 8)), (D, D, (0, 4, 6, 7, 8)))
F32 = jnp.float32
BF16 = jnp.bfloat16
U32 = jnp.uint32


def _consts():
    ang = 2.0 * np.pi * np.outer(np.arange(T) + 0.25, np.arange(T)) / T
    fwd = np.stack([np.cos(ang), np.sin(ang)], axis=1)
    fwd = fwd.reshape(2, T // 16, 8, 2, T).transpose(1, 0, 3, 2, 4).reshape(2 * T, T)
    inv = np.stack([np.cos(ang), np.sin(ang)], axis=1)[:T // 2].reshape(T, T).T / T
    inv = np.concatenate([inv[0::2], inv[1::2]], axis=0)
    lane = np.arange(128) // DH
    head_mask = (lane[:, None] == lane[None, :]).astype(np.float32)
    return [a.astype(np.float32).astype(BF16) for a in (fwd, inv, head_mask)]


def _phi(t):
    return jnp.where(t > 0, t + 1.0, jnp.exp(t)) + 1e-6


def _recip(d):
    r = pl.reciprocal(d, approx=True)
    return r * (2.0 - d * r)


def _aligned(i, n):
    return i if isinstance(i, int) else pl.multiple_of(i, n)


def _pack(x):
    return pltpu.bitcast(x, U32)


def _unpack(x):
    return pltpu.bitcast(x, BF16)


def _split(w):
    return [pltpu.unpack_elementwise(w, index=i, packed_dtype=BF16, unpacked_dtype=F32) for i in range(2)]


def _merge(even, odd):
    return pltpu.pack_elementwise([even, odd], packed_dtype=BF16)


def _dot_t(a, b):
    return lax.dot_general(a, b, (((1,), (1,)), ((), ())), preferred_element_type=F32)


def _dot(a, b):
    return jnp.dot(a, b, preferred_element_type=F32)


def _kernel(x_h, wqkv_h, wo_h, q_h, k_h, v_h, sk_h, ssm_h, d_h, fwd_h, inv_h, msk_h, out_h,
           x_v, wk_v, wq_v, wv_v, wo_v, q_v, k_v, v_v, sk_v, ssm_v, d_v, fwd_v, inv_v, msk_v,
           fu_v, gu_v, kf_v, pk0_v, pk1_v, pacc_v, p_v, z_v, wqt_v, zc_v, pq0_v, pq1_v, m_v, oa_v, ob_v, sems, bar, *rest):
    kv_v, xs_v, ks_v, zs_v = rest[0:3], rest[3:5], rest[5:7], rest[7:9]
    sem_ids = {}

    def copy(name, src, dst):
        if name not in sem_ids:
            sem_ids[name] = len(sem_ids)
        return pltpu.make_async_copy(src, dst, sems.at[sem_ids[name]])

    d_row = lambda g: d_v[...].astype(F32)[g * 128:(g + 1) * 128].reshape(1, 128)
    cols = lambda g: pl.ds(g * 128, 128)
    xw_v, ku_v, vu_v, qu_v, obu_v = [r.bitcast(U32) for r in (x_v, k_v, v_v, q_v, ob_v)]
    XC = 256
    cp_x = [[copy(("x", r0, g), x_h.at[pl.ds(r0, n), cols(g)], x_v.at[g, pl.ds(r0, n)]) for g in range(NG)]
            for r0, n in ((0, XC), (XC, XC), (2 * XC, 2 * XC), (4 * XC, S - 4 * XC))]
    cp_wk = [copy(("wk", g), wqkv_h.at[:, pl.ds(D + g * 128, 128)], wk_v.at[g]) for g in range(NG)]
    cp_wq = copy("wq", wqkv_h.at[:, pl.ds(0, D)], wq_v)
    cp_wv = copy("wv", wqkv_h.at[:, pl.ds(2 * D, D)], wv_v)
    cp_wo = copy("wo", wo_h, wo_v)
    cp_q = [copy(("q", g), q_h.at[:, cols(g)], q_v.at[g]) for g in range(NG)]
    cp_k = [copy(("k", g), k_h.at[:, cols(g)], k_v.at[g]) for g in range(NG)]
    cp_v = [copy(("v", g), v_h.at[:, cols(g)], v_v.at[g]) for g in range(NG)]
    cp_s = [copy(("s", g), ssm_h.at[cols(g)], ssm_v.at[g]) for g in range(NG)]
    cp_sk, cp_d, cp_fwd = copy("sk", sk_h, sk_v), copy("d", d_h, d_v), copy("fwd", fwd_h, fwd_v)
    cp_inv, cp_msk = copy("inv", inv_h, inv_v), copy("msk", msk_h, msk_v)
    cp_ob = [copy(("ob", g), ob_v.at[g], out_h.at[:, pl.ds(D + g * 128, 128)]) for g in range(NG)]
    cp_oa = [[copy(("oa", r0, c0), oa_v.at[pl.ds(r0, n), pl.ds(c0 * 128, (c1 - c0) * 128)],
                   out_h.at[pl.ds(r0, n), pl.ds(c0 * 128, (c1 - c0) * 128)]) for c0, c1 in zip(cc, cc[1:])]
             for r0, n, cc in OUT_PIECES]

    class Plan:
        def __init__(self, nslots):
            self.keep = msk_v[0:8, :].astype(F32) > -1.0
            self.load = [0.0] * nslots
            self.items = [[] for _ in range(nslots)]
            self.pos = 0

        def put(self, slot, cost, fn):
            slot = min(slot, len(self.load) - 1)
            self.load[slot] += cost
            self.items[slot].append(fn)

        def spread(self, lo, hi, items):
            for n, (cost, fn) in enumerate(items):
                self.put(lo + (n * (hi - lo)) // len(items), cost, fn)

        def fill(self, lo, hi, items):
            total = sum(c for c, _ in items)
            level = (total + sum(self.load[lo:hi])) / (hi - lo)
            while sum(max(level - l, 0.0) for l in self.load[lo:hi]) > total:
                level -= 0.25
            slot, room = lo, 0.0
            room = max(level - self.load[lo], 0.0)
            for cost, fn in items:
                while room < cost / 2 and slot < hi - 1:
                    slot += 1
                    room += max(level - self.load[slot], 0.0)
                room -= cost
                self.put(slot, cost, fn)

        def slab(self, val, step):
            toks = []
            for _ in range(step):
                for fn in self.items[self.pos]:
                    toks += fn()
                self.pos += 1
            if not toks:
                return val
            for tk in toks:
                val = jnp.where(self.keep, val, tk if tk.dtype == U32 else pltpu.bitcast(tk, U32))
            return val

        def lhs(self, val, step=1):
            m, k = val.shape
            parts = []
            for c in range(0, k, 512):
                parts.append(jnp.concatenate(
                    [self.slab(val[r:r + 8, c:c + 128], step) for r in range(0, m, 8)], axis=0))
                if min(c + 512, k) > c + 128:
                    parts.append(val[:, c + 128:min(c + 512, k)])
            return _unpack(parts[0] if len(parts) == 1 else jnp.concatenate(parts, axis=1))

        def finish(self):
            assert self.pos == len(self.load) - 1, (self.pos, len(self.load))
            for fn in self.items[self.pos]:
                fn()

    zeros = []

    def rows_at(r0, n, salt):
        return pl.ds(pl.multiple_of(r0 + zeros[salt % len(zeros)], 8), n)

    def pre_items(g, it, kvs):
        w = sk_v[:, cols(g)].astype(F32)
        w0, w1, w2, w3 = [jnp.broadcast_to(w[tau:tau + 1], (8, 128)) for tau in range(KS)]

        def item(n):
            def fn():
                r0 = it * T + n * 8
                for r in range(0 if r0 == 0 else r0 + 8, min(r0 + 16, S // 2), 8):
                    for j, kk in enumerate(_split(ku_v[g, pl.ds(r, 8), :])):
                        kf_v[j, pl.ds(HALO + r, 8), :] = kk
                ve, vo = _split(vu_v[g, pl.ds(r0, 8), :])
                ke = kf_v[0, pl.ds(HALO + r0, 8), :]
                ko = kf_v[1, pl.ds(HALO + r0, 8), :]
                ke1 = kf_v[0, pl.ds(HALO + r0 - 1, 8), :]
                ko1 = kf_v[1, pl.ds(HALO + r0 - 1, 8), :]
                ko2 = kf_v[1, pl.ds(HALO + r0 - 2, 8), :]
                se = (ke * w0 + ko1 * w1) + (ke1 * w2 + ko2 * w3)
                so = (ko * w0 + ke * w1) + (ko1 * w2 + ke1 * w3)
                kv = _merge(se * ve, so * vo)
                kv_v[g % 3][pl.ds(r0, 8), :] = kv
                kvs.append(kv)
                return [kv]
            return (22, fn)
        return [item(n) for n in range(2 * T // 16)]

    def fwd_filter(g, it, plan):
        flt = jnp.concatenate([ssm_v[g, :, pl.ds((it * 4 + b) * T, T)] for b in range(4)], axis=0)
        res = _dot_t(plan.lhs(fu_v[rows_at(0, T, it), :]), flt)
        for b in range(4):
            ks_v[g % 2][it * 4 + b] = res[:, b * 128:(b + 1) * 128]

    def fwd_data(g, it, kvs, plan):
        dat = jnp.concatenate([jnp.concatenate(kvs[b * 8:(b + 1) * 8], axis=0) for b in range(4)], axis=1)
        res = _dot(plan.lhs(fu_v[rows_at(0, T, it + 4), :]), _unpack(dat))
        for b in range(4):
            xs_v[g % 2][it * 4 + b] = res[:, b * 128:(b + 1) * 128]

    def mac_items(g, it):
        s = g % 2
        items, low = [], []
        for pp in range(2):
            st = dict(res=[[], []])
            for part in range(3):
                for i in range(NB):
                    def fn(pp=pp, part=part, i=i, st=st):
                        r0 = (it * 2 + pp) * 16

                        def operand(ref):
                            vals = [ref[i, pl.ds(r0 + 8 * c, 8), :] for c in ((0,), (1,), (0, 1))[part]]
                            return vals[0] if part < 2 else vals[0] + vals[1]

                        if i == 0:
                            st['k'], st['x'] = [], []
                        st['k'].append(operand(ks_v[s]))
                        st['x'].append(operand(xs_v[s]))
                        acc = st['k'][i] * st['x'][0]
                        for j in range(1, i + 1):
                            acc = acc + st['k'][i - j] * st['x'][j]
                        if part < 2:
                            st['res'][part].append(acc)
                            return [acc]
                        p1, p2 = st['res'][0][i], st['res'][1][i]
                        yr, yi = p1 - p2, acc - (p1 + p2)
                        zr = yr if i == 0 else yr + st['yi']
                        zi = yi if i == 0 else yi - st['yr']
                        st['yr'], st['yi'] = yr, yi
                        if pp == 0:
                            low.append((zr, zi))
                            return [zr if i % 2 else zi]
                        ar, ai = low[i]
                        ze, zo = _merge(ar + zr, ai + zi), _merge(ar - zr, ai - zi)
                        zs_v[s][i, pl.ds(it * 8, 8), :] = ze
                        zs_v[s][i, pl.ds(T // 2 + it * 8, 8), :] = zo
                        return [zo if i % 2 else ze]
                    items.append((2 * i + 2 + (7 + 6 * pp if part == 2 else 0), fn))
        return items

    def inv_dots(g, it, plan):
        ys = []
        for n in range(8):
            half = (n % 2) * (T // 2)
            gm = gu_v[rows_at(half // 2, T // 4, it * 8 + n), :]
            ys.append(_dot(plan.lhs(gm) if n % 4 == 0 else _unpack(gm),
                           _unpack(zs_v[g % 2][it * 4 + n // 2, pl.ds(half, T // 2), :])))
        return ys

    def inv_items(g, it, ys):
        dd = jnp.broadcast_to(d_row(g), (8, 128))

        def item(n):
            def fn():
                rows = pl.ds(it * 2 * T + n * 8, 8)
                ye, yo = [ys[(n // 8) * 2 + j][(n % 8) * 8:(n % 8 + 1) * 8] for j in range(2)]
                kve, kvo = _split(kv_v[g % 3][rows, :])
                qe, qo = _split(qu_v[g, rows, :])
                ob = _merge(qe * (ye + kve * dd), qo * (yo + kvo * dd))
                obu_v[g, rows, :] = ob
                return [ob]
            return (12, fn)
        return [item(n) for n in range(4 * T // 16)]

    def lanes(it, base=0):
        return pl.ds(base + it * 128, 128)

    def a_k(r0, mc, it, plan):
        st = {}
        rows = rows_at(r0 // 2, mc // 2, it)
        xu = jnp.concatenate([xw_v[g, rows, :] for g in range(NG)], axis=1)
        res = _dot(plan.lhs(xu), _unpack(wk_v.bitcast(U32)[it]))
        pks = []

        def item(n):
            def fn():
                pk = _phi(res[n * 16:(n + 1) * 16])
                part = pk[0:8] + pk[8:16]
                st['z'] = part if 'z' not in st else st['z'] + part
                pks.append(pk)
                if n % 8 < 7:
                    return [part]
                pkt = jnp.concatenate(pks[-8:], axis=0).astype(BF16).T
                (pk0_v, pk1_v)[r0 // D][pl.ds(it * 64, 64), pl.ds(r0 % D + (n // 8) * 128, 128)] = _pack(pkt)
                if n == mc // 16 - 1:
                    z_v[it] = st['z'] if r0 == 0 else z_v[it] + st['z']
                return [part]
            return (20, fn)
        return [item(n) for n in range(mc // 16)]

    def a_p(s0, mc, it, plan):
        res = _dot(plan.lhs((pk0_v, pk1_v)[s0 // D][rows_at(0, D // 2, it), :]),
                   _unpack(xw_v[it, pl.ds(s0 // 2, S // 4), :]))

        def item(n):
            def fn():
                part = res[n * 16:(n + 1) * 16]
                if s0 == 0:
                    pacc_v[it, pl.ds(n * 16, 16), :] = part
                    return []
                part = part + pacc_v[it, pl.ds(n * 16, 16), :]
                pb = _merge(part[0:8], part[8:16])
                p_v[pl.ds(n * 8, 8), lanes(it)] = pb
                return []
            return (2, fn)
        return [item(n) for n in range(mc // 16)]

    def prep_items(h, it):
        def wq(n):
            def fn():
                r0 = h * (D // 2) + n * 128
                blk = _pack(wq_v[pl.ds(r0, 128), lanes(it)].T)
                wqt_v[pl.ds(it * 64, 64), pl.ds(r0, 128)] = blk
                return [blk[56:64]]
            return (4, fn)

        def zc():
            z = jnp.sum(z_v[it], axis=0, keepdims=True)
            col = jnp.broadcast_to(z, (128, 128)).T
            zc_v[lanes(it), :] = col
            return [col[120:128]]
        return [wq(n) for n in range(4)] if h < 2 else [(8, zc)]

    def a_q(f0, mc, it, plan):
        rows = pl.ds(it % 8 * 64, 64)
        xr = rows_at(it * 64, 64, f0 // mc)
        xu = jnp.concatenate([xw_v[g, xr, :] for g in range(NG)], axis=1)
        res = _dot_t(plan.lhs(wqt_v[rows_at(f0 // 2, mc // 2, it), :]), _unpack(xu))
        outs = []

        def item(n):
            def fn():
                pq = _phi(res[n * DH:(n + 1) * DH])
                pz = pq * zc_v[pl.ds(f0 + n * DH, DH), :]
                den = (pz[0:8] + pz[8:16]) + (pz[16:24] + pz[24:32])
                for sh in (4, 2, 1):
                    den = den + pltpu.roll(den, sh, 0)
                inv = _recip(den + 1e-6)
                pqn = pq * jnp.concatenate([inv] * 4, axis=0)
                outs.extend([_merge(pqn[0:8], pqn[8:16]), _merge(pqn[16:24], pqn[24:32])])
                if n % 4 == 3:
                    (pq0_v, pq1_v)[it // 8][rows, pl.ds(f0 + (n // 4) * 128, 128)] = _pack(_unpack(jnp.concatenate(outs[-8:], axis=0)).T)
                return outs[-2:]
            return (56, fn)
        return [item(n) for n in range(mc // DH)]

    def a_o(r0, mc, it, plan):
        res = _dot(plan.lhs((pq0_v, pq1_v)[r0 // D][rows_at(0, mc // 2, it), :]), m_v[:, lanes(it)])

        def item(n):
            def fn():
                ob = res[n * 16:(n + 1) * 16].astype(BF16)
                oa_v[pl.ds(r0 + n * 16, 16), lanes(it)] = ob
                return []
            return (2, fn)
        return [item(n) for n in range(mc // 16)]

    a_fn = dict(k=a_k, p=a_p, q=a_q, o=a_o)
    a_cost = dict(k=20 / 16, p=2 / 16, q=28 / 16, o=2 / 16)

    kvs = {}

    def block(work, vec):
        pl.semaphore_signal(bar, 1)
        pl.semaphore_wait(bar, 1)
        work = sorted(work, key=lambda e: e[0])
        seq = [e for _, e in work]
        start, n = [], 0
        for e in seq:
            start.append(n)
            n += e[2] // 8 if e[0] in a_fn else dict(kv=16, m=16, inv=8, ff=16, fd=16, dma=0)[e[0]]
        start.append(n)
        slot_at = lambda t: start[sum(1 for tt, _ in work if tt < t)]
        plan = Plan(n + 1)
        late, prev = {}, 0
        for i, e in enumerate(seq):
            lo = min(start[i + 1] + LAG, n)
            if e[0] == 'inv':
                late[i] = (lo, min(lo + 48, n + 1), 12 * 32)
            elif e[0] in a_fn:
                late[i] = (lo, min(lo + e[2] // 8, n + 1), a_cost[e[0]] * e[2])
            elif e[0] == 'fd':
                kvs[e[1:]] = []
                items = sum([pre_items(e[1], 2 * e[2] + j, kvs[e[1:]]) for j in range(2)], [])
                lo = max(prev, start[i] - 160)
                plan.spread(lo, max(start[i] - 8, lo + 1), items)
                prev = start[i]
        for lo, hi, cost in late.values():
            for sl in range(lo, hi):
                plan.load[sl] += cost / (hi - lo)
        for items, first, last, even in vec:
            (plan.spread if even else plan.fill)(slot_at(first), max(slot_at(last), slot_at(first) + 1), items)
        done = [0]

        def place(i, items):
            lo, hi, cost = late[i]
            for sl in range(lo, hi):
                plan.load[sl] -= cost / (hi - lo)
            plan.spread(lo, hi, items)
            done[0] = max(done[0], hi - 1)

        for i, e in enumerate(seq):
            if e[0] == 'kv':
                kvh = _dot(plan.lhs(p_v[pl.ds(e[1] * 64, 64), :]), wv_v[:, lanes(e[1])])
                kvs['head', e[1]] = _pack(jnp.where(msk_v[...] > 0, kvh, 0.0).astype(BF16))
            elif e[0] == 'm':
                for c in range(2):
                    half = pl.ds(c * (D // 2), D // 2)
                    m_v[lanes(e[1]), half] = _dot(plan.lhs(kvs['head', e[1]]), wo_v[lanes(e[1]), half]).astype(BF16)
            elif e[0] == 'inv':
                place(i, inv_items(e[1], e[2], inv_dots(e[1], e[2], plan)))
            elif e[0] == 'ff':
                fwd_filter(e[1], e[2], plan)
            elif e[0] == 'fd':
                fwd_data(e[1], e[2], kvs[e[1], e[2]], plan)
            elif e[0] == 'dma':
                plan.put(max(done[0], plan.pos), 0, lambda c=e[1]: (c.start(), [])[1])
            else:
                place(i, a_fn[e[0]](e[1], e[2], e[3], plan))
        plan.finish()

    def a_work():
        unit = lambda kind, h: [[(kind, h * D, D, it)] for it in range(8)]
        q = [[('q', 0, D, it)] for it in range(16)]
        o = [unit('o', h) for h in range(2)]
        for (_, _, cc), cps, oh in zip(OUT_PIECES, cp_oa, o):
            for c1, cp in zip(cc[1:], cps):
                oh[c1 - 1].append(('dma', cp))
        res = [(r0 / 128 + it * mc / D, ('k', r0, mc, it))
               for r0, mc in ((0, XC), (XC, XC), (2 * XC, D - 2 * XC)) for it in range(8)]
        mix = lambda a, b: [u for pair in zip(a, b) for u in pair]
        units = mix(unit('k', 1), unit('p', 0)) + mix(unit('p', 1), q[:8]) + q[8:10]
        units += mix(o[0][:6], q[10:]) + o[0][6:] + o[1]
        res += [(8 + t + j / 2, e) for t, es in enumerate(units) for j, e in enumerate(es)]
        return res + spread(40.1, 41.9, [('kv', 0)] + sum(
            [[('kv', g + 1), ('m', g)] for g in range(NG - 1)], []) + [('m', NG - 1)])

    def spread(t0, t1, es):
        return [(t0 + (n + 0.5) * (t1 - t0) / len(es), e) for n, e in enumerate(es)]

    def all_macs(g):
        return sum([mac_items(g, it) for it in range(8)], [])

    grp = lambda g: [cp_s[g], cp_k[g], cp_v[g]]
    ff = lambda g: [('ff', g, it) for it in range(4)]
    fd = lambda g: [('fd', g, it) for it in range(4)]
    inv = lambda g: [('inv', g, it) for it in range(4)] + [('dma', cp_ob[g])]

    def clusters(t0, t1, kinds):
        groups = [[k[it] for k in kinds] for it in range(4)]
        return [(t + 0.01 * j, e) for t, es in spread(t0, t1, groups) for j, e in enumerate(es)]

    tb, c0, c1 = GROUP_TIMES, 3.5, 5.5
    work, vec = a_work(), []
    work += spread(c0, c0 + 0.2, ff(0)) + spread(c0 + 0.3, 4, fd(0)) + clusters(c1, tb[1], [ff(1), fd(1)])
    for g in range(NG):
        t0, t1 = tb[g], tb[g + 1]
        if 1 <= g < NG - 1:
            work += clusters(t0 + 0.1, t1 + 0.1, [fd(g + 1), inv(g - 1), ff(g + 1)])
            work += [(t1 - 0.1, inv(g - 1)[4])]
        vec.append((all_macs(g), t0, t1, False))
    work += clusters(tb[7], tb[8] - 1, [inv(6)]) + [(tb[8] - 1, inv(6)[4])]
    work += clusters(tb[8], tb[9] - 0.4, [inv(7)]) + [(tb[9] - 0.2, inv(7)[4])]
    vec.append((sum([prep_items(h, it) for h in range(2) for it in range(8)], []), tb[2] + 0.1, 23.9, True))
    vec.append((sum([prep_items(2, it) for it in range(8)], []), 24.1, 25.5, True))

    cuts = [(j / 4, cp_wk[j:j + 2]) for j in range(0, NG, 2)]
    cuts[0] = (0, [cp_msk] + cp_x[0] + cuts[0][1])
    cuts += [(2, cp_x[1]), (c0, [cp_fwd, cp_sk] + grp(0)), (4, cp_x[2]), (c1, grp(1)),
             (8, cp_x[3]), (tb[1], [cp_inv, cp_d, cp_q[0]] + grp(2)),
             (tb[2], [cp_q[1], cp_wq] + grp(3) + [cp_q[2]] + grp(4)),
             (tb[3], [cp_q[3]] + grp(5)), (tb[4], cp_q[4:] + [cp_wv, cp_wo] + grp(6) + grp(7))]
    cuts += [(t, []) for t in tb[5:8]]
    cuts.sort(key=lambda c: c[0])
    ready = lambda cp: next(t for t, need in cuts if any(c is cp for c in need))
    for t, e in work:
        uses = dict(ff=lambda g, _: [cp_fwd, cp_s[g]], fd=lambda g, _: [cp_sk, cp_k[g], cp_v[g]],
                    inv=lambda g, _: [cp_inv, cp_d, cp_q[g]], kv=lambda g: [cp_wv], m=lambda g: [cp_wo])
        assert all(ready(cp) <= t for cp in uses.get(e[0], lambda *_: [])(*e[1:])), (t, e)
    assert ready(cp_wq) <= tb[2] and ready(cp_x[3][0]) <= 8
    for _, need in cuts:
        for c in need:
            c.start()
    kf_v[:, pl.ds(0, HALO), :] = jnp.zeros((2, HALO, 128), F32)
    for (t0, need), t1 in zip(cuts, [t for t, _ in cuts[1:]] + [65]):
        for c in need:
            c.wait()
        if t0 == 0:
            zv = jnp.where(msk_v[0:16, :].astype(F32) > -1.0, 0, 1)
            zeros.extend(zv[i, 0] for i in range(16))
        if t0 == c0:
            fu_v[...] = _pack(fwd_v[...])
        if any(c is cp_inv for c in need):
            gu_v[...] = _pack(inv_v[...])
        part = []
        for items, f, l, even in vec:
            lo, hi = max(t0, f), min(t1, l)
            if lo < hi:
                cut = lambda t: round(len(items) * (t - f) / (l - f))
                part.append((items[cut(lo):cut(hi)], lo, hi, even))
        if t1 > t0:
            block([e for e in work if t0 <= e[0] < t1], part)
    for c in cp_ob + sum(cp_oa, []):
        c.wait()

@jax.jit
def pallas_concat_heads__linear_attn_block__ssm_conv_h3__prompt_kernel(
    A_x, A_wqkv, A_wo, B_q, B_k, B_v, B_shift_k, B_ssm_k, B_ssm_D):
    fwd, inv, msk = _consts()
    any_spec = pl.BlockSpec(memory_space=pl.ANY)
    vm = pltpu.VMEM
    out = pl.pallas_call(
        _kernel,
        out_shape=jax.ShapeDtypeStruct((S, 2 * D), BF16),
        in_specs=[any_spec] * 12,
        out_specs=any_spec,
        scratch_shapes=[
            vm((NG, S, 128), BF16), vm((NG, D, 128), BF16), vm((D, D), BF16), vm((D, D), BF16), vm((D, D), BF16),
            vm((NG, S, 128), BF16), vm((NG, S, 128), BF16), vm((NG, S, 128), BF16),
            vm((KS, D), BF16), vm((NG, 128, S), BF16), vm((D,), BF16),
            vm((2 * T, T), BF16), vm((T, T), BF16), vm((128, 128), BF16),
            vm((T, T), U32), vm((T // 2, T), U32), vm((2, HALO + S // 2, 128), F32),
            vm((D // 2, S // 2), U32), vm((D // 2, S // 2), U32), vm((NG, D, 128), F32), vm((D // 2, D), U32), vm((NG, 8, 128), F32), vm((D // 2, D), U32), vm((D, 128), F32),
            vm((S // 4, D), U32), vm((S // 4, D), U32), vm((D, D), BF16), vm((S, D), BF16), vm((NG, S, 128), BF16),
            pltpu.SemaphoreType.DMA((104,)), pltpu.SemaphoreType.REGULAR,
        ] + [vm((S // 2, 128), U32)] * 3 + [vm((NB, 2 * T, 128), F32)] * 4 + [vm((NB, T, 128), U32)] * 2,
        compiler_params=pltpu.CompilerParams(vmem_limit_bytes=100 * 1024 * 1024),
    )(A_x.reshape(S, D), A_wqkv, A_wo, B_q.reshape(S, D), B_k.reshape(S, D), B_v.reshape(S, D),
      B_shift_k.T, B_ssm_k, B_ssm_D,
      fwd, inv, msk)
    return out.reshape(1, S, 2 * D)
```

```python
import numpy as np
import jax
import jax.numpy as jnp
from jax import lax
from jax.experimental import pallas as pl
from jax.experimental.pallas import tpu as pltpu

S = 2048
D = 1024
DH = 32
T = 128
NB = S // T
NG = D // 128
KS = 4
HALO = 8
LAG = 3
GROUP_TIMES = (4, 11, 18, 26, 34, 42, 50, 57, 61.5, 63)
FIRST_TRANSFORMS = (3.5, 5.5)
OUT_PIECES = ((0, D, (0, 8)), (D, D, (0, 5, 7, 8)))
F32 = jnp.float32
BF16 = jnp.bfloat16
U32 = jnp.uint32


def _consts():
    ang = 2.0 * np.pi * np.outer(np.arange(T) + 0.25, np.arange(T)) / T
    fwd = np.stack([np.cos(ang), np.sin(ang)], axis=1)
    fwd = fwd.reshape(2, T // 16, 8, 2, T).transpose(1, 0, 3, 2, 4).reshape(2 * T, T)
    inv = np.stack([np.cos(ang), np.sin(ang)], axis=1)[:T // 2].reshape(T, T).T / T
    inv = np.concatenate([inv[0::2], inv[1::2]], axis=0)
    lane = np.arange(128) // DH
    head_mask = (lane[:, None] == lane[None, :]).astype(np.float32)
    return [a.astype(np.float32).astype(BF16) for a in (fwd, inv, head_mask)]


def _phi(t):
    return jnp.where(t > 0, t + 1.0, jnp.exp(t)) + 1e-6


def _recip(d):
    r = pl.reciprocal(d, approx=True)
    return r * (2.0 - d * r)


def _pack(x):
    return pltpu.bitcast(x, U32)


def _unpack(x):
    return pltpu.bitcast(x, BF16)


def _split(w):
    return [pltpu.unpack_elementwise(w, index=i, packed_dtype=BF16, unpacked_dtype=F32) for i in range(2)]


def _merge(even, odd):
    return pltpu.pack_elementwise([even, odd], packed_dtype=BF16)


def _dot_t(a, b):
    return lax.dot_general(a, b, (((1,), (1,)), ((), ())), preferred_element_type=F32)


def _dot(a, b):
    return jnp.dot(a, b, preferred_element_type=F32)


def _kernel(x_h, wqkv_h, wo_h, q_h, k_h, v_h, sk_h, ssm_h, d_h, fwd_h, inv_h, msk_h, out_h,
           x_v, wk_v, wq_v, wv_v, wo_v, q_v, k_v, v_v, sk_v, ssm_v, d_v, fwd_v, inv_v, msk_v,
           fu_v, gu_v, kf_v, pk0_v, pk1_v, pacc_v, p_v, z_v, wqt_v, zc_v, pq0_v, pq1_v, m_v, oa_v, ob_v, sems, bar, *rest):
    kv_v, xs_v, ks_v, zs_v = rest[0:3], rest[3:5], rest[5:7], rest[7:9]
    sem_ids = {}

    def copy(name, src, dst):
        if name not in sem_ids:
            sem_ids[name] = len(sem_ids)
        return pltpu.make_async_copy(src, dst, sems.at[sem_ids[name]])

    d_row = lambda g: d_v[...].astype(F32)[g * 128:(g + 1) * 128].reshape(1, 128)
    cols = lambda g: pl.ds(g * 128, 128)
    xw_v, ku_v, vu_v, qu_v, obu_v = [r.bitcast(U32) for r in (x_v, k_v, v_v, q_v, ob_v)]
    XC = 256
    cp_x = [[copy(("x", r0, g), x_h.at[pl.ds(r0, n), cols(g)], x_v.at[g, pl.ds(r0, n)]) for g in range(NG)]
            for r0, n in ((0, XC), (XC, XC), (2 * XC, 2 * XC), (4 * XC, S - 4 * XC))]
    cp_wk = [copy(("wk", g), wqkv_h.at[:, pl.ds(D + g * 128, 128)], wk_v.at[g]) for g in range(NG)]
    cp_wq = copy("wq", wqkv_h.at[:, pl.ds(0, D)], wq_v)
    cp_wv = copy("wv", wqkv_h.at[:, pl.ds(2 * D, D)], wv_v)
    cp_wo = copy("wo", wo_h, wo_v)
    cp_q = [copy(("q", g), q_h.at[:, cols(g)], q_v.at[g]) for g in range(NG)]
    cp_k = [copy(("k", g), k_h.at[:, cols(g)], k_v.at[g]) for g in range(NG)]
    cp_v = [copy(("v", g), v_h.at[:, cols(g)], v_v.at[g]) for g in range(NG)]
    cp_s = [copy(("s", g), ssm_h.at[cols(g)], ssm_v.at[g]) for g in range(NG)]
    cp_sk, cp_d, cp_fwd = copy("sk", sk_h, sk_v), copy("d", d_h, d_v), copy("fwd", fwd_h, fwd_v)
    cp_inv, cp_msk = copy("inv", inv_h, inv_v), copy("msk", msk_h, msk_v)
    cp_ob = [copy(("ob", g), ob_v.at[g], out_h.at[:, pl.ds(D + g * 128, 128)]) for g in range(NG)]
    cp_oa = [[copy(("oa", r0, c0), oa_v.at[pl.ds(r0, n), pl.ds(c0 * 128, (c1 - c0) * 128)],
                   out_h.at[pl.ds(r0, n), pl.ds(c0 * 128, (c1 - c0) * 128)]) for c0, c1 in zip(cc, cc[1:])]
             for r0, n, cc in OUT_PIECES]

    class Plan:
        def __init__(self, nslots):
            self.keep = msk_v[0:8, :].astype(F32) > -1.0
            self.load = [0.0] * nslots
            self.items = [[] for _ in range(nslots)]
            self.pos = 0

        def put(self, slot, cost, fn):
            slot = min(slot, len(self.load) - 1)
            self.load[slot] += cost
            self.items[slot].append(fn)

        def spread(self, lo, hi, items):
            for n, (cost, fn) in enumerate(items):
                self.put(lo + (n * (hi - lo)) // len(items), cost, fn)

        def fill(self, lo, hi, items):
            total = sum(c for c, _ in items)
            level = (total + sum(self.load[lo:hi])) / (hi - lo)
            while sum(max(level - l, 0.0) for l in self.load[lo:hi]) > total:
                level -= 0.25
            slot, room = lo, 0.0
            room = max(level - self.load[lo], 0.0)
            for cost, fn in items:
                while room < cost / 2 and slot < hi - 1:
                    slot += 1
                    room += max(level - self.load[slot], 0.0)
                room -= cost
                self.put(slot, cost, fn)

        def slab(self, val, step):
            toks = []
            for _ in range(step):
                for fn in self.items[self.pos]:
                    toks += fn()
                self.pos += 1
            if not toks:
                return val
            for tk in toks:
                val = jnp.where(self.keep, val, tk if tk.dtype == U32 else pltpu.bitcast(tk, U32))
            return val

        def lhs(self, val, step=1):
            m, k = val.shape
            parts = []
            for c in range(0, k, 512):
                parts.append(jnp.concatenate(
                    [self.slab(val[r:r + 8, c:c + 128], step) for r in range(0, m, 8)], axis=0))
                if min(c + 512, k) > c + 128:
                    parts.append(val[:, c + 128:min(c + 512, k)])
            return _unpack(parts[0] if len(parts) == 1 else jnp.concatenate(parts, axis=1))

        def finish(self):
            assert self.pos == len(self.load) - 1, (self.pos, len(self.load))
            for fn in self.items[self.pos]:
                fn()

    zeros = []

    def rows_at(r0, n, salt):
        return pl.ds(pl.multiple_of(r0 + zeros[salt % len(zeros)], 8), n)

    def pre_items(g, it, kvs):
        w = sk_v[:, cols(g)].astype(F32)
        w0, w1, w2, w3 = [jnp.broadcast_to(w[tau:tau + 1], (8, 128)) for tau in range(KS)]

        def item(n):
            def fn():
                r0 = it * T + n * 8
                for r in range(0 if r0 == 0 else r0 + 8, min(r0 + 16, S // 2), 8):
                    for j, kk in enumerate(_split(ku_v[g, pl.ds(r, 8), :])):
                        kf_v[j, pl.ds(HALO + r, 8), :] = kk
                ve, vo = _split(vu_v[g, pl.ds(r0, 8), :])
                ke = kf_v[0, pl.ds(HALO + r0, 8), :]
                ko = kf_v[1, pl.ds(HALO + r0, 8), :]
                ke1 = kf_v[0, pl.ds(HALO + r0 - 1, 8), :]
                ko1 = kf_v[1, pl.ds(HALO + r0 - 1, 8), :]
                ko2 = kf_v[1, pl.ds(HALO + r0 - 2, 8), :]
                se = (ke * w0 + ko1 * w1) + (ke1 * w2 + ko2 * w3)
                so = (ko * w0 + ke * w1) + (ko1 * w2 + ke1 * w3)
                kv = _merge(se * ve, so * vo)
                kv_v[g % 3][pl.ds(r0, 8), :] = kv
                kvs.append(kv)
                return [kv]
            return (22, fn)
        return [item(n) for n in range(2 * T // 16)]

    def fwd_filter(g, it, plan):
        flt = jnp.concatenate([ssm_v[g, :, pl.ds((it * 4 + b) * T, T)] for b in range(4)], axis=0)
        res = _dot_t(plan.lhs(fu_v[rows_at(0, T, it), :]), flt)
        for b in range(4):
            ks_v[g % 2][it * 4 + b] = res[:, b * 128:(b + 1) * 128]

    def fwd_data(g, it, kvs, plan):
        dat = jnp.concatenate([jnp.concatenate(kvs[b * 8:(b + 1) * 8], axis=0) for b in range(4)], axis=1)
        res = _dot(plan.lhs(fu_v[rows_at(0, T, it + 4), :]), _unpack(dat))
        for b in range(4):
            xs_v[g % 2][it * 4 + b] = res[:, b * 128:(b + 1) * 128]

    def mac_items(g, it):
        s = g % 2
        items, low = [], []
        for pp in range(2):
            st = dict(res=[[], []])
            for part in range(3):
                for i in range(NB):
                    def fn(pp=pp, part=part, i=i, st=st):
                        r0 = (it * 2 + pp) * 16

                        def operand(ref):
                            vals = [ref[i, pl.ds(r0 + 8 * c, 8), :] for c in ((0,), (1,), (0, 1))[part]]
                            return vals[0] if part < 2 else vals[0] + vals[1]

                        if i == 0:
                            st['k'], st['x'] = [], []
                        st['k'].append(operand(ks_v[s]))
                        st['x'].append(operand(xs_v[s]))
                        acc = st['k'][i] * st['x'][0]
                        for j in range(1, i + 1):
                            acc = acc + st['k'][i - j] * st['x'][j]
                        if part < 2:
                            st['res'][part].append(acc)
                            return [acc]
                        p1, p2 = st['res'][0][i], st['res'][1][i]
                        yr, yi = p1 - p2, acc - (p1 + p2)
                        zr = yr if i == 0 else yr + st['yi']
                        zi = yi if i == 0 else yi - st['yr']
                        st['yr'], st['yi'] = yr, yi
                        if pp == 0:
                            low.append((zr, zi))
                            return [zr if i % 2 else zi]
                        ar, ai = low[i]
                        ze, zo = _merge(ar + zr, ai + zi), _merge(ar - zr, ai - zi)
                        zs_v[s][i, pl.ds(it * 8, 8), :] = ze
                        zs_v[s][i, pl.ds(T // 2 + it * 8, 8), :] = zo
                        return [zo if i % 2 else ze]
                    items.append((2 * i + 2 + (7 + 6 * pp if part == 2 else 0), fn))
        return items

    def inv_dots(g, it, plan):
        ys = []
        for n in range(8):
            half = (n % 2) * (T // 2)
            gm = gu_v[rows_at(half // 2, T // 4, it * 8 + n), :]
            ys.append(_dot(plan.lhs(gm) if n % 4 == 0 else _unpack(gm),
                           _unpack(zs_v[g % 2][it * 4 + n // 2, pl.ds(half, T // 2), :])))
        return ys

    def inv_items(g, it, ys):
        dd = jnp.broadcast_to(d_row(g), (8, 128))

        def item(n):
            def fn():
                rows = pl.ds(it * 2 * T + n * 8, 8)
                ye, yo = [ys[(n // 8) * 2 + j][(n % 8) * 8:(n % 8 + 1) * 8] for j in range(2)]
                kve, kvo = _split(kv_v[g % 3][rows, :])
                qe, qo = _split(qu_v[g, rows, :])
                ob = _merge(qe * (ye + kve * dd), qo * (yo + kvo * dd))
                obu_v[g, rows, :] = ob
                return [ob]
            return (12, fn)
        return [item(n) for n in range(4 * T // 16)]

    def lanes(it):
        return pl.ds(it * 128, 128)

    def a_k(r0, mc, it, plan):
        st = {}
        rows = rows_at(r0 // 2, mc // 2, it)
        xu = jnp.concatenate([xw_v[g, rows, :] for g in range(NG)], axis=1)
        res = _dot(plan.lhs(xu), _unpack(wk_v.bitcast(U32)[it]))
        pks = []

        def item(n):
            def fn():
                pk = _phi(res[n * 16:(n + 1) * 16])
                part = pk[0:8] + pk[8:16]
                st['z'] = part if 'z' not in st else st['z'] + part
                pks.append(pk)
                if n % 8 < 7:
                    return [part]
                pkt = jnp.concatenate(pks[-8:], axis=0).astype(BF16).T
                (pk0_v, pk1_v)[r0 // D][pl.ds(it * 64, 64), pl.ds(r0 % D + (n // 8) * 128, 128)] = _pack(pkt)
                if n == mc // 16 - 1:
                    z_v[it] = st['z'] if r0 == 0 else z_v[it] + st['z']
                return [part]
            return (20, fn)
        return [item(n) for n in range(mc // 16)]

    def a_p(s0, mc, it, plan):
        res = _dot(plan.lhs((pk0_v, pk1_v)[s0 // D][rows_at(0, D // 2, it), :]),
                   _unpack(xw_v[it, pl.ds(s0 // 2, S // 4), :]))

        def item(n):
            def fn():
                part = res[n * 16:(n + 1) * 16]
                if s0 == 0:
                    pacc_v[it, pl.ds(n * 16, 16), :] = part
                    return []
                part = part + pacc_v[it, pl.ds(n * 16, 16), :]
                pb = _merge(part[0:8], part[8:16])
                p_v[pl.ds(n * 8, 8), lanes(it)] = pb
                return []
            return (2, fn)
        return [item(n) for n in range(mc // 16)]

    def prep_items(h, it):
        def wq(n):
            def fn():
                r0 = h * (D // 2) + n * 128
                blk = _pack(wq_v[pl.ds(r0, 128), lanes(it)].T)
                wqt_v[pl.ds(it * 64, 64), pl.ds(r0, 128)] = blk
                return [blk[56:64]]
            return (4, fn)

        def zc():
            z = jnp.sum(z_v[it], axis=0, keepdims=True)
            col = jnp.broadcast_to(z, (128, 128)).T
            zc_v[lanes(it), :] = col
            return [col[120:128]]
        return [wq(n) for n in range(4)] if h < 2 else [(8, zc)]

    def a_q(f0, mc, it, plan):
        rows = pl.ds(it % 8 * 64, 64)
        xr = rows_at(it * 64, 64, f0 // mc)
        xu = jnp.concatenate([xw_v[g, xr, :] for g in range(NG)], axis=1)
        res = _dot_t(plan.lhs(wqt_v[rows_at(f0 // 2, mc // 2, it), :]), _unpack(xu))
        outs = []

        def item(n):
            def fn():
                pq = _phi(res[n * DH:(n + 1) * DH])
                pz = pq * zc_v[pl.ds(f0 + n * DH, DH), :]
                den = (pz[0:8] + pz[8:16]) + (pz[16:24] + pz[24:32])
                for sh in (4, 2, 1):
                    den = den + pltpu.roll(den, sh, 0)
                inv = _recip(den + 1e-6)
                pqn = pq * jnp.concatenate([inv] * 4, axis=0)
                outs.extend([_merge(pqn[0:8], pqn[8:16]), _merge(pqn[16:24], pqn[24:32])])
                if n % 4 == 3:
                    (pq0_v, pq1_v)[it // 8][rows, pl.ds(f0 + (n // 4) * 128, 128)] = _pack(_unpack(jnp.concatenate(outs[-8:], axis=0)).T)
                return outs[-2:]
            return (56, fn)
        return [item(n) for n in range(mc // DH)]

    def a_o(r0, mc, it, plan):
        res = _dot(plan.lhs((pq0_v, pq1_v)[r0 // D][rows_at(0, mc // 2, it), :]), m_v[:, lanes(it)])

        def item(n):
            def fn():
                ob = res[n * 16:(n + 1) * 16].astype(BF16)
                oa_v[pl.ds(r0 + n * 16, 16), lanes(it)] = ob
                return []
            return (2, fn)
        return [item(n) for n in range(mc // 16)]

    a_fn = dict(k=a_k, p=a_p, q=a_q, o=a_o)
    a_cost = dict(k=20 / 16, p=2 / 16, q=28 / 16, o=2 / 16)

    kvs = {}

    def block(work, vec):
        pl.semaphore_signal(bar, 1)
        pl.semaphore_wait(bar, 1)
        work = sorted(work, key=lambda e: e[0])
        seq = [e for _, e in work]
        start, n = [], 0
        for e in seq:
            start.append(n)
            n += e[2] // 8 if e[0] in a_fn else dict(kv=16, m=16, inv=8, ff=16, fd=16, dma=0)[e[0]]
        start.append(n)
        slot_at = lambda t: start[sum(1 for tt, _ in work if tt < t)]
        plan = Plan(n + 1)
        late, prev = {}, 0
        for i, e in enumerate(seq):
            lo = min(start[i + 1] + LAG, n)
            if e[0] == 'inv':
                late[i] = (lo, min(lo + 48, n + 1), 12 * 32)
            elif e[0] in a_fn:
                late[i] = (lo, min(lo + e[2] // 8, n + 1), a_cost[e[0]] * e[2])
            elif e[0] == 'fd':
                kvs[e[1:]] = []
                items = sum([pre_items(e[1], 2 * e[2] + j, kvs[e[1:]]) for j in range(2)], [])
                lo = max(prev, start[i] - 160)
                plan.spread(lo, max(start[i] - 8, lo + 1), items)
                prev = start[i]
        for lo, hi, cost in late.values():
            for sl in range(lo, hi):
                plan.load[sl] += cost / (hi - lo)
        for items, first, last, even in vec:
            (plan.spread if even else plan.fill)(slot_at(first), max(slot_at(last), slot_at(first) + 1), items)
        done = [0]

        def place(i, items):
            lo, hi, cost = late[i]
            for sl in range(lo, hi):
                plan.load[sl] -= cost / (hi - lo)
            plan.spread(lo, hi, items)
            done[0] = max(done[0], hi - 1)

        for i, e in enumerate(seq):
            if e[0] == 'kv':
                kvh = _dot(plan.lhs(p_v[pl.ds(e[1] * 64, 64), :]), wv_v[:, lanes(e[1])])
                kvs['head', e[1]] = _pack(jnp.where(msk_v[...] > 0, kvh, 0.0).astype(BF16))
            elif e[0] == 'm':
                for c in range(2):
                    half = pl.ds(c * (D // 2), D // 2)
                    m_v[lanes(e[1]), half] = _dot(plan.lhs(kvs['head', e[1]]), wo_v[lanes(e[1]), half]).astype(BF16)
            elif e[0] == 'inv':
                place(i, inv_items(e[1], e[2], inv_dots(e[1], e[2], plan)))
            elif e[0] == 'ff':
                fwd_filter(e[1], e[2], plan)
            elif e[0] == 'fd':
                fwd_data(e[1], e[2], kvs[e[1], e[2]], plan)
            elif e[0] == 'dma':
                plan.put(max(done[0], plan.pos), 0, lambda c=e[1]: (c.start(), [])[1])
            else:
                place(i, a_fn[e[0]](e[1], e[2], e[3], plan))
        plan.finish()

    def a_work():
        unit = lambda kind, h: [[(kind, h * D, D, it)] for it in range(8)]
        q = [[('q', 0, D, it)] for it in range(16)]
        o = [unit('o', h) for h in range(2)]
        for (_, _, cc), cps, oh in zip(OUT_PIECES, cp_oa, o):
            for c1, cp in zip(cc[1:], cps):
                oh[c1 - 1].append(('dma', cp))
        res = [(r0 / 128 + it * mc / D, ('k', r0, mc, it))
               for r0, mc in ((0, XC), (XC, XC), (2 * XC, D - 2 * XC)) for it in range(8)]
        mix = lambda a, b: [u for pair in zip(a, b) for u in pair]
        units = mix(unit('k', 1), unit('p', 0)) + mix(unit('p', 1), q[:8]) + q[8:10]
        units += mix(o[0][:6], q[10:]) + o[0][6:] + o[1]
        res += [(8 + t + j / 2, e) for t, es in enumerate(units) for j, e in enumerate(es)]
        return res + spread(40.1, 41.9, [('kv', 0)] + sum(
            [[('kv', g + 1), ('m', g)] for g in range(NG - 1)], []) + [('m', NG - 1)])

    def spread(t0, t1, es):
        return [(t0 + (n + 0.5) * (t1 - t0) / len(es), e) for n, e in enumerate(es)]

    def all_macs(g):
        return sum([mac_items(g, it) for it in range(8)], [])

    grp = lambda g: [cp_s[g], cp_k[g], cp_v[g]]
    ff = lambda g: [('ff', g, it) for it in range(4)]
    fd = lambda g: [('fd', g, it) for it in range(4)]
    inv = lambda g: [('inv', g, it) for it in range(4)] + [('dma', cp_ob[g])]

    def clusters(t0, t1, kinds):
        groups = [[k[it] for k in kinds] for it in range(4)]
        return [(t + 0.01 * j, e) for t, es in spread(t0, t1, groups) for j, e in enumerate(es)]

    tb, (c0, c1) = GROUP_TIMES, FIRST_TRANSFORMS
    work, vec = a_work(), []
    work += spread(c0, c0 + 0.2, ff(0)) + spread(c0 + 0.3, 4, fd(0)) + clusters(c1, tb[1], [ff(1), fd(1)])
    for g in range(NG):
        t0, t1 = tb[g], tb[g + 1]
        if 1 <= g < NG - 1:
            work += clusters(t0 + 0.1, t1 + 0.1, [fd(g + 1), inv(g - 1), ff(g + 1)])
            work += [(t1 - 0.1, inv(g - 1)[4])]
        vec.append((all_macs(g), t0, t1, False))
    work += clusters(tb[7], tb[8] - 1, [inv(6)]) + [(tb[8] - 1, inv(6)[4])]
    work += clusters(tb[8], tb[9] - 0.4, [inv(7)]) + [(tb[9] - 0.2, inv(7)[4])]
    vec.append((sum([prep_items(h, it) for h in range(2) for it in range(8)], []), tb[2] + 0.1, 23.9, True))
    vec.append((sum([prep_items(2, it) for it in range(8)], []), 24.1, 25.5, True))

    cuts = [(j / 4, cp_wk[j:j + 2]) for j in range(0, NG, 2)]
    cuts[0] = (0, [cp_msk] + cp_x[0] + cuts[0][1])
    cuts += [(2, cp_x[1]), (c0, [cp_fwd, cp_sk] + grp(0)), (4, cp_x[2]), (c1, grp(1)),
             (8, cp_x[3]), (tb[1], [cp_inv, cp_d, cp_q[0]] + grp(2)),
             (tb[2], [cp_q[1], cp_wq] + grp(3) + [cp_q[2]] + grp(4)),
             (tb[3], [cp_q[3]] + grp(5)), (tb[4], cp_q[4:] + [cp_wv, cp_wo] + grp(6) + grp(7))]
    cuts += [(t, []) for t in tb[5:8]]
    cuts.sort(key=lambda c: c[0])
    ready = lambda cp: next(t for t, need in cuts if any(c is cp for c in need))
    for t, e in work:
        uses = dict(ff=lambda g, _: [cp_fwd, cp_s[g]], fd=lambda g, _: [cp_sk, cp_k[g], cp_v[g]],
                    inv=lambda g, _: [cp_inv, cp_d, cp_q[g]], kv=lambda g: [cp_wv], m=lambda g: [cp_wo])
        assert all(ready(cp) <= t for cp in uses.get(e[0], lambda *_: [])(*e[1:])), (t, e)
    assert ready(cp_wq) <= tb[2] and ready(cp_x[3][0]) <= 8
    for _, need in cuts:
        for c in need:
            c.start()
    kf_v[:, pl.ds(0, HALO), :] = jnp.zeros((2, HALO, 128), F32)
    for (t0, need), t1 in zip(cuts, [t for t, _ in cuts[1:]] + [65]):
        for c in need:
            c.wait()
        if t0 == 0:
            zv = jnp.where(msk_v[0:16, :].astype(F32) > -1.0, 0, 1)
            zeros.extend(zv[i, 0] for i in range(16))
        if t0 == c0:
            fu_v[...] = _pack(fwd_v[...])
        if any(c is cp_inv for c in need):
            gu_v[...] = _pack(inv_v[...])
        part = []
        for items, f, l, even in vec:
            lo, hi = max(t0, f), min(t1, l)
            if lo < hi:
                cut = lambda t: round(len(items) * (t - f) / (l - f))
                part.append((items[cut(lo):cut(hi)], lo, hi, even))
        if t1 > t0:
            block([e for e in work if t0 <= e[0] < t1], part)
    for c in cp_ob + sum(cp_oa, []):
        c.wait()

@jax.jit
def pallas_concat_heads__linear_attn_block__ssm_conv_h3__prompt_kernel(
    A_x, A_wqkv, A_wo, B_q, B_k, B_v, B_shift_k, B_ssm_k, B_ssm_D):
    fwd, inv, msk = _consts()
    any_spec = pl.BlockSpec(memory_space=pl.ANY)
    vm = pltpu.VMEM
    out = pl.pallas_call(
        _kernel,
        out_shape=jax.ShapeDtypeStruct((S, 2 * D), BF16),
        in_specs=[any_spec] * 12,
        out_specs=any_spec,
        scratch_shapes=[
            vm((NG, S, 128), BF16), vm((NG, D, 128), BF16), vm((D, D), BF16), vm((D, D), BF16), vm((D, D), BF16),
            vm((NG, S, 128), BF16), vm((NG, S, 128), BF16), vm((NG, S, 128), BF16),
            vm((KS, D), BF16), vm((NG, 128, S), BF16), vm((D,), BF16),
            vm((2 * T, T), BF16), vm((T, T), BF16), vm((128, 128), BF16),
            vm((T, T), U32), vm((T // 2, T), U32), vm((2, HALO + S // 2, 128), F32),
            vm((D // 2, S // 2), U32), vm((D // 2, S // 2), U32), vm((NG, D, 128), F32), vm((D // 2, D), U32), vm((NG, 8, 128), F32), vm((D // 2, D), U32), vm((D, 128), F32),
            vm((S // 4, D), U32), vm((S // 4, D), U32), vm((D, D), BF16), vm((S, D), BF16), vm((NG, S, 128), BF16),
            pltpu.SemaphoreType.DMA((104,)), pltpu.SemaphoreType.REGULAR,
        ] + [vm((S // 2, 128), U32)] * 3 + [vm((NB, 2 * T, 128), F32)] * 4 + [vm((NB, T, 128), U32)] * 2,
        compiler_params=pltpu.CompilerParams(vmem_limit_bytes=100 * 1024 * 1024),
    )(A_x.reshape(S, D), A_wqkv, A_wo, B_q.reshape(S, D), B_k.reshape(S, D), B_v.reshape(S, D),
      B_shift_k.T, B_ssm_k, B_ssm_D,
      fwd, inv, msk)
    return out.reshape(1, S, 2 * D)
```
